```python
import jax
import jax.numpy as jnp

def _softmax(x, axis=-1):
    return jax.nn.softmax(x, axis=axis)

def _gelu(x):
    return jax.nn.gelu(x, approximate=True)

def _silu(x):
    return jax.nn.silu(x)

def _sigmoid(x):
    return jax.nn.sigmoid(x)

def _layernorm(x, axis=-1, eps=1e-05):
    m = jnp.mean(x, axis=axis, keepdims=True)
    v = jnp.var(x, axis=axis, keepdims=True)
    return (x - m) / jnp.sqrt(v + eps)

def _scatter_add(tgt, idx, src, axis=0):
    return tgt.at[idx].add(src)

def _segment_sum(src, seg, n):
    return jax.ops.segment_sum(src, seg, n)

class _Rng:

    def __init__(self, key):
        self._k = key

    def _next(self):
        self._k, sub = jax.random.split(self._k)
        return sub

    def normal(self, shape):
        return jax.random.normal(self._next(), shape, dtype=jnp.bfloat16)

    def randint(self, lo, hi, shape):
        return jax.random.randint(self._next(), shape, lo, hi, dtype=jnp.int32)

    def uniform(self, shape, lo=0.0, hi=1.0):
        return jax.random.uniform(self._next(), shape, jnp.bfloat16, lo, hi)

    def permutation(self, n):
        return jax.random.permutation(self._next(), n)
kernel_name = 'adaLN_cond__gqa_block_cached__moe_arch_mod__prompt'

def setup_inputs():
    _rng = _Rng(jax.random.key(int.from_bytes(__import__("os").urandom(4), "little")))
    _w = lambda a: (lambda t: t.astype(jnp.bfloat16) if jnp.issubdtype(t.dtype, jnp.floating) else t)(jnp.asarray(a))

    def _A_setup():
        B, Sq, D = (1, 2048, 576)
        Hq, Hkv, Sk, Dh = (32, 16, 2048, 128)
        assert Hq % Hkv == 0, (Hq, Hkv)
        return {'x': _w((lambda *s: _rng.normal(s) * 0.05)(B, Sq, D)), 'k_cache': _w((lambda *s: _rng.normal(s) * 0.05)(B, Hkv, Sk, Dh)), 'v_cache': _w((lambda *s: _rng.normal(s) * 0.05)(B, Hkv, Sk, Dh)), 'wq': _w((lambda *s: _rng.normal(s) * 0.05)(D, Hq * Dh) * D ** (-0.5)), 'wo': _w((lambda *s: _rng.normal(s) * 0.05)(Hq * Dh, D) * (Hq * Dh) ** (-0.5))}
    _A_in = _A_setup()

    def _B_setup():
        B, S, D, F, C = (1, 2048, 576, 4608, 8)
        return {'x': _w((lambda *s: _rng.normal(s) * 0.05)(B, S, D)), 'w_r': _w((lambda *s: _rng.normal(s) * 0.05)(D)), 'w_gate': _w((lambda *s: _rng.normal(s) * 0.05)(D, F)), 'w_up': _w((lambda *s: _rng.normal(s) * 0.05)(D, F)), 'w_down': _w((lambda *s: _rng.normal(s) * 0.05)(F, D))}
    _B_in = _B_setup()
    return {'A_x': _A_in['x'], 'A_k_cache': _A_in['k_cache'], 'A_v_cache': _A_in['v_cache'], 'A_wq': _A_in['wq'], 'A_wo': _A_in['wo'], 'B_x': _B_in['x'], 'B_w_r': _B_in['w_r'], 'B_w_gate': _B_in['w_gate'], 'B_w_up': _B_in['w_up'], 'B_w_down': _B_in['w_down'], 'c': _w((lambda *s: _rng.normal(s) * 0.05)(1, 576)), 'w_mod': _w((lambda *s: _rng.normal(s) * 0.05)(576, 6 * 576) * 576 ** (-0.5))}

def reference(A_x, A_k_cache, A_v_cache, A_wq, A_wo, B_x, B_w_r, B_w_gate, B_w_up, B_w_down, c, w_mod):

    def _A_ref(x, k_cache, v_cache, wq, wo):
        B, Sq, D = x.shape
        Hq, Dh = (32, 128)
        Hkv = k_cache.shape[1]
        rep = Hq // Hkv
        q = (lambda x, *d: x.transpose(*d))((x @ wq).reshape(B, Sq, Hq, Dh), 0, 2, 1, 3)
        k = jnp.repeat(k_cache, rep, axis=1)
        v = jnp.repeat(v_cache, rep, axis=1)
        scores = jnp.einsum('bhqd,bhkd->bhqk', q, k) * Dh ** (-0.5)
        p = _softmax(scores, axis=-1)
        o = jnp.einsum('bhqk,bhkd->bhqd', p, v)
        return (lambda x, *d: x.transpose(*d))(o, 0, 2, 1, 3).reshape(B, Sq, Hq * Dh) @ wo

    def _B_ref(x, w_r, w_gate, w_up, w_down):
        B, S, D = x.shape
        C = 8
        r = x @ w_r
        idx = jnp.argsort(-r, axis=-1)[:, :C]
        idx_e = jnp.repeat(idx.reshape(B, C, 1), D, axis=2)
        x_sel = jnp.take_along_axis(x, idx_e, axis=1)
        g = _silu(x_sel @ w_gate)
        u = x_sel @ w_up
        y = g * u @ w_down
        r_sel = _sigmoid(jnp.take_along_axis(r, idx, axis=1))
        y = y * r_sel.reshape(B, C, 1)
        b_off = (jnp.arange(B) * S).reshape(B, 1)
        flat_idx = (idx + b_off).reshape(B * C)
        zero = (x * 0.0).reshape(B * S, D)
        upd = _scatter_add(zero, flat_idx, y.reshape(B * C, D), axis=0)
        return x + upd.reshape(B, S, D)
    x = A_x
    mod = (_silu(c) @ w_mod).reshape(c.shape[0], 6, 1, -1)
    sa, ca, ga, sb, cb, gb = (mod[:, 0].copy(), mod[:, 1].copy(), mod[:, 2].copy(), mod[:, 3].copy(), mod[:, 4].copy(), mod[:, 5].copy())
    h = _layernorm(x, axis=-1) * (1 + ca) + sa
    x = x + ga * _A_ref(h, A_k_cache, A_v_cache, A_wq, A_wo)
    h = _layernorm(x, axis=-1) * (1 + cb) + sb
    x = x + gb * _B_ref(h, B_w_r, B_w_gate, B_w_up, B_w_down)
    return x
```

```python
import functools
import math

import jax
import jax.numpy as jnp
import numpy as np
from jax import lax
from jax.experimental import pallas as pl
from jax.experimental.pallas import tpu as pltpu

S = 2048
D = 576
HQ = 32
HKV = 16
DH = 128
F = 4608
TOPK = 8
EPS = 1e-5

R_ATT = 256
R_LN = 256
R_OP = 256

F32 = jnp.float32
BF16 = jnp.bfloat16
NT_DIMS = (((1,), (1,)), ((), ()))
NN_DIMS = (((1,), (0,)), ((), ()))


def _rb(v):
    return v.astype(BF16).astype(F32)


def _dot(a, b, dims=NN_DIMS):
    return lax.dot_general(a, b, dims, preferred_element_type=F32)


def _sigmoid_b(g):
    return _rb(1.0 / _rb(1.0 + _rb(jnp.exp(-g))))


def _ln_t(xf):
    inv_d = np.float32(1.0 / D)
    m32 = jnp.sum(xf, axis=0, keepdims=True) * inv_d
    cen = xf - m32
    v = _rb(jnp.sum(cen * cen, axis=0, keepdims=True) * inv_d)
    eps_b = np.float32(np.float32(EPS).astype(jnp.bfloat16))
    den = _rb(jnp.sqrt(_rb(v + eps_b)))
    inv = 1.0 / den
    return _rb(_rb(xf - _rb(m32)) * inv)


def _col(row):
    return jnp.broadcast_to(row, (128, D)).T


def _kernel(xt_hbm, k_hbm, v_hbm, wq_hbm, wot_hbm, wr_hbm, wg_hbm, wu_hbm, wdt_hbm, c_hbm, wmod_hbm,
            out_hbm,
            x_buf, h_buf, k_buf, v_buf, wq_buf, wo_buf, wr_buf, wg_buf, wu_buf, wd_buf, c_buf,
            wma_buf, wmb_buf, o_buf, x1_buf, h2_buf, out_buf, r_buf, xs_buf, idx_smem,
            sem_misc, sem_k, sem_v, sem_q, sem_out):
    def cp(src, dst, sem):
        return pltpu.make_async_copy(src, dst, sem)

    d_c = cp(c_hbm, c_buf, sem_misc.at[0])
    d_wma = cp(wmod_hbm.at[:, pl.ds(0, 2 * D)], wma_buf, sem_misc.at[1])
    d_x = cp(xt_hbm, x_buf, sem_misc.at[2])
    d_wmb = cp(wmod_hbm.at[:, pl.ds(2 * D, 4 * D)], wmb_buf, sem_misc.at[3])
    d_wo = cp(wot_hbm, wo_buf, sem_misc.at[4])
    d_wr = cp(wr_hbm, wr_buf, sem_misc.at[5])
    d_wg = cp(wg_hbm, wg_buf, sem_misc.at[6])
    d_wu = cp(wu_hbm, wu_buf, sem_misc.at[7])
    d_wd = cp(wdt_hbm, wd_buf, sem_misc.at[8])

    def d_k(j):
        return cp(k_hbm.at[j], k_buf.at[j], sem_k.at[j])

    def d_v(j):
        return cp(v_hbm.at[j], v_buf.at[j], sem_v.at[j])

    def d_q(j):
        return cp(wq_hbm.at[:, pl.ds(pl.multiple_of(j * 2 * DH, 2 * DH), 2 * DH)], wq_buf.at[j], sem_q.at[j])

    d_c.start()
    d_wma.start()
    d_x.start()
    d_q(0).start()
    d_k(0).start()
    d_v(0).start()

    d_c.wait()
    cf = c_buf[...].astype(F32)
    sc = _rb(cf * _sigmoid_b(cf))
    sc8 = jnp.broadcast_to(sc, (8, D)).astype(BF16)
    d_wma.wait()
    mod_a = _rb(_dot(sc8, wma_buf[...]))
    sa = mod_a[0:1, 0:D]
    ca1 = _rb(1.0 + mod_a[0:1, D:2 * D])

    d_x.wait()

    def ln1_body(b, carry):
        t0 = pl.multiple_of(b * R_LN, R_LN)
        xf = x_buf[:, pl.ds(t0, R_LN)].astype(F32)
        ln = _ln_t(xf).T
        h_buf[pl.ds(t0, R_LN), :] = _rb(_rb(ln * ca1) + sa).astype(BF16)
        return carry

    lax.fori_loop(0, S // R_LN, ln1_body, 0)

    q_scale = np.float32(DH ** -0.5 * math.log2(math.e))

    def att_body(j, carry):
        @pl.when(j + 1 < HKV)
        def _():
            d_q(j + 1).start()
            d_k(j + 1).start()
            d_v(j + 1).start()

        @pl.when(j == 0)
        def _():
            d_wmb.start()
            d_wr.start()

        @pl.when(j == 1)
        def _():
            d_wo.start()

        @pl.when(j == 2)
        def _():
            d_wg.start()

        @pl.when(j == 3)
        def _():
            d_wu.start()

        @pl.when(j == 4)
        def _():
            d_wd.start()

        d_q(j).wait()
        d_k(j).wait()
        d_v(j).wait()
        for b in range(S // R_ATT):
            rows = pl.ds(b * R_ATT, R_ATT)
            q2 = (_dot(h_buf[rows, :], wq_buf[j]) * q_scale).astype(BF16)
            for hh in range(2):
                q = q2[:, hh * DH:(hh + 1) * DH]
                s = _dot(q, k_buf[j], NT_DIMS)
                m = jnp.max(s, axis=-1, keepdims=True)
                p = jnp.exp2(s - m)
                l = jnp.sum(p, axis=-1, keepdims=True)
                o = _dot(p.astype(BF16), v_buf[j])
                o_buf[2 * j + hh, rows, :] = (o * pltpu.reciprocal(l, approx=True)).astype(BF16)
        return carry

    lax.fori_loop(0, HKV, att_body, 0)

    d_wmb.wait()
    mod_b = _rb(_dot(sc8, wmb_buf[...]))
    gb = mod_b[0:1, 3 * D:4 * D]
    ga_c = _col(mod_b[0:1, 0:D])
    sb_c = _col(mod_b[0:1, D:2 * D])
    cb1_c = _col(_rb(1.0 + mod_b[0:1, 2 * D:3 * D]))
    gb_c = _col(gb)
    d_wr.wait()
    wr_c = _col(wr_buf[...].astype(F32).reshape(1, D))
    d_wo.wait()

    def op_body(b, carry):
        t0 = pl.multiple_of(b * R_OP, R_OP)
        toks = pl.ds(t0, R_OP)
        o_cat = jnp.concatenate([o_buf[h, toks, :] for h in range(HQ)], axis=1)
        attn_all = _rb(_dot(wo_buf[...], o_cat, NT_DIMS))
        for t in range(R_OP // 128):
            tk = pl.ds(t0 + t * 128, 128)
            attn = attn_all[:, t * 128:(t + 1) * 128]
            x1 = _rb(x_buf[:, tk].astype(F32) + _rb(ga_c * attn))
            h2 = _rb(_rb(_ln_t(x1) * cb1_c) + sb_c)
            r_buf[pl.ds(b * (R_OP // 128) + t, 1), :] = _rb(jnp.sum(h2 * wr_c, axis=0, keepdims=True))
            hb = _rb(h2 + _rb(h2 * 0.0))
            out_buf[:, tk] = (x1 + _rb(gb_c * hb)).astype(BF16)
            x1_buf[tk, :] = x1.T
            h2_buf[tk, :] = h2.T
        return carry

    lax.fori_loop(0, S // R_OP, op_body, 0)

    r_all = r_buf[...]
    neg_inf = np.float32(-np.inf)
    lowest = np.float32(np.finfo(np.float32).min)
    key = jnp.where(r_all != r_all, neg_inf, jnp.maximum(r_all, lowest))
    pos = (lax.broadcasted_iota(jnp.int32, (S // 128, 128), 0) * 128
           + lax.broadcasted_iota(jnp.int32, (S // 128, 128), 1)).astype(F32)
    live = jnp.ones((S // 128, 128), F32)
    r_sel = jnp.zeros((TOPK, 1), F32)
    sel_row = lax.broadcasted_iota(jnp.int32, (TOPK, 1), 0)
    for t in range(TOPK):
        m = jnp.max(jnp.where(live > 0, key, neg_inf))
        cand = jnp.logical_and(key == m, live > 0)
        pf = jnp.min(jnp.where(cand, pos, np.float32(S - 1)))
        hit = pos == pf
        live = jnp.where(hit, 0.0, live)
        idx_smem[t] = pf.astype(jnp.int32)
        r_sel = jnp.where(sel_row == t, jnp.sum(jnp.where(hit, r_all, 0.0)), r_sel)

    for t in range(TOPK):
        xs_buf[pl.ds(t, 1), :] = h2_buf[pl.ds(idx_smem[t], 1), :]
        xs_buf[pl.ds(TOPK + t, 1), :] = x1_buf[pl.ds(idx_smem[t], 1), :]
    xs = xs_buf[0:TOPK, :]
    xs_b = xs.astype(BF16)

    d_wg.wait()
    d_wu.wait()
    g = _rb(_dot(xs_b, wg_buf[...]))
    u = _rb(_dot(xs_b, wu_buf[...]))
    act = _rb(_rb(g * _sigmoid_b(g)) * u).astype(BF16)
    d_wd.wait()
    y = _rb(_dot(act, wd_buf[...], NT_DIMS))
    y = _rb(y * _sigmoid_b(r_sel))
    hb_sel = _rb(xs + _rb(_rb(xs * 0.0) + y))
    new = xs_buf[TOPK:2 * TOPK, :] + _rb(gb * hb_sel)
    new_t = jnp.concatenate([new, jnp.zeros((128 - TOPK, D), F32)], axis=0).T

    lane = lax.broadcasted_iota(jnp.int32, (D, 128), 1)
    for t in range(TOPK):
        i = idx_smem[t]
        blk = pl.ds(pl.multiple_of((i // 128) * 128, 128), 128)
        colv = jnp.broadcast_to(new_t[:, t:t + 1], (D, 128))
        out_buf[:, blk] = jnp.where(lane == i % 128, colv, out_buf[:, blk].astype(F32)).astype(BF16)

    d_out = cp(out_buf, out_hbm, sem_out)
    d_out.start()
    d_out.wait()


@jax.jit
def pallas_adaLN_cond__gqa_block_cached__moe_arch_mod__prompt_kernel(
    A_x, A_k_cache, A_v_cache, A_wq, A_wo, B_x, B_w_r, B_w_gate, B_w_up, B_w_down, c, w_mod,
):
    del B_x
    xt = A_x.reshape(S, D).T
    k = A_k_cache.reshape(HKV, S, DH)
    v = A_v_cache.reshape(HKV, S, DH)
    hbm = pl.BlockSpec(memory_space=pl.ANY)
    out = pl.pallas_call(
        _kernel,
        in_specs=[hbm] * 11,
        out_specs=hbm,
        out_shape=jax.ShapeDtypeStruct((D, S), BF16),
        scratch_shapes=[
            pltpu.VMEM((D, S), BF16),
            pltpu.VMEM((S, D), BF16),
            pltpu.VMEM((HKV, S, DH), BF16),
            pltpu.VMEM((HKV, S, DH), BF16),
            pltpu.VMEM((HKV, D, 2 * DH), BF16),
            pltpu.VMEM((D, HQ * DH), BF16),
            pltpu.VMEM((D,), BF16),
            pltpu.VMEM((D, F), BF16),
            pltpu.VMEM((D, F), BF16),
            pltpu.VMEM((D, F), BF16),
            pltpu.VMEM((1, D), BF16),
            pltpu.VMEM((D, 2 * D), BF16),
            pltpu.VMEM((D, 4 * D), BF16),
            pltpu.VMEM((HQ, S, DH), BF16),
            pltpu.VMEM((S, D), F32),
            pltpu.VMEM((S, D), F32),
            pltpu.VMEM((D, S), BF16),
            pltpu.VMEM((S // 128, 128), F32),
            pltpu.VMEM((2 * TOPK, D), F32),
            pltpu.SMEM((TOPK,), jnp.int32),
            pltpu.SemaphoreType.DMA((9,)),
            pltpu.SemaphoreType.DMA((HKV,)),
            pltpu.SemaphoreType.DMA((HKV,)),
            pltpu.SemaphoreType.DMA((HKV,)),
            pltpu.SemaphoreType.DMA,
        ],
        compiler_params=pltpu.CompilerParams(vmem_limit_bytes=120 * 1024 * 1024),
    )(xt, k, v, A_wq, A_wo.T, B_w_r, B_w_gate, B_w_up, B_w_down.T, c, w_mod)
    return out.T.reshape(1, S, D)
```

```python
import functools
import math

import jax
import jax.numpy as jnp
import numpy as np
from jax import lax
from jax.experimental import pallas as pl
from jax.experimental.pallas import tpu as pltpu

S = 2048
D = 576
HQ = 32
HKV = 16
DH = 128
F = 4608
TOPK = 8
EPS = 1e-5
TB = 128
NTB = S // TB
NP = (D + 127) // 128

R_ATT = 256
R_LN = 256
OP_UNROLL = 3

F32 = jnp.float32
BF16 = jnp.bfloat16
NT_DIMS = (((1,), (1,)), ((), ()))
NN_DIMS = (((1,), (0,)), ((), ()))


def _rb(v):
    return v.astype(BF16).astype(F32)


def _dot(a, b, dims=NN_DIMS):
    return lax.dot_general(a, b, dims, preferred_element_type=F32)


def _sigmoid_b(g):
    return _rb(1.0 / _rb(1.0 + _rb(jnp.exp(-g))))


def _ln_t(xf):
    inv_d = np.float32(1.0 / D)
    m32 = jnp.sum(xf, axis=0, keepdims=True) * inv_d
    cen = xf - m32
    v = _rb(jnp.sum(cen * cen, axis=0, keepdims=True) * inv_d)
    eps_b = np.float32(np.float32(EPS).astype(jnp.bfloat16))
    den = _rb(jnp.sqrt(_rb(v + eps_b)))
    inv = 1.0 / den
    return _rb(_rb(xf - _rb(m32)) * inv)


def _col(row):
    return jnp.broadcast_to(row, (128, D)).T


KEY_BIAS = 0x20000000


def _sort_key(r, tok):
    bits = lax.bitcast_convert_type(r, jnp.int32)
    u = lax.shift_right_logical(bits, 16)
    u = jnp.where(u == 0x8000, 0, u)
    srt = jnp.where(u >= 0x8000, 0xFFFF - u, u | 0x8000)
    srt = jnp.where(r != r, 0, srt)
    key = lax.shift_left(srt, 11) | (S - 1 - tok)
    return lax.bitcast_convert_type(key + KEY_BIAS, F32)


def _kernel(xt_hbm, k_hbm, v_hbm, wq_hbm, wot_hbm, wr_hbm, wg_hbm, wu_hbm, wdt_hbm, c_hbm, wmod_hbm,
            out_hbm,
            x_buf, h_buf, k_buf, v_buf, wq_buf, wo_buf, wr_buf, wg_buf, wu_buf, wd_buf, c_buf,
            wma_buf, wmb_buf, o_buf, x1_buf, h2_buf, out_buf, key_buf, att_buf, xs_buf, idx_smem,
            sem_misc, sem_k, sem_v, sem_q, sem_x, sem_out, sem_patch):
    k32 = k_buf.bitcast(jnp.int32)
    v32 = v_buf.bitcast(jnp.int32)
    o32 = o_buf.bitcast(jnp.int32)
    h32 = h_buf.bitcast(jnp.int32)
    wo32 = wo_buf.bitcast(jnp.int32)

    def as_bf16(v):
        return pltpu.bitcast(v, BF16)

    def cp(src, dst, sem):
        return pltpu.make_async_copy(src, dst, sem)

    d_c = cp(c_hbm, c_buf, sem_misc.at[0])
    d_wma = cp(wmod_hbm.at[:, pl.ds(0, 2 * D)], wma_buf, sem_misc.at[1])
    d_wmb = cp(wmod_hbm.at[:, pl.ds(2 * D, 4 * D)], wmb_buf, sem_misc.at[3])

    class _Group:
        def __init__(self, copies):
            self.copies = copies

        def start(self):
            for c in self.copies:
                c.start()

        def wait(self):
            for c in self.copies:
                c.wait()

    d_wo = _Group([cp(wot_hbm.at[:, pl.ds(h * DH, DH)], wo_buf.at[h], sem_misc.at[4]) for h in range(HQ)])
    d_wr = cp(wr_hbm, wr_buf, sem_misc.at[5])
    d_wg = cp(wg_hbm, wg_buf, sem_misc.at[6])
    d_wu = cp(wu_hbm, wu_buf, sem_misc.at[7])
    d_wd = cp(wdt_hbm, wd_buf, sem_misc.at[8])

    def d_x(b):
        return cp(xt_hbm.at[:, pl.ds(pl.multiple_of(b * TB, TB), TB)], x_buf.at[b], sem_x.at[b])

    def d_out(b):
        return cp(out_buf.at[b], out_hbm.at[:, pl.ds(pl.multiple_of(b * TB, TB), TB)], sem_out.at[b])

    def d_k(jj):
        return cp(k_hbm.at[pl.ds(2 * jj, 2)], k_buf.at[pl.ds(2 * jj, 2)], sem_k.at[jj])

    def d_v(jj):
        return cp(v_hbm.at[pl.ds(2 * jj, 2)], v_buf.at[pl.ds(2 * jj, 2)], sem_v.at[jj])

    def d_q(jj):
        return cp(wq_hbm.at[:, pl.ds(pl.multiple_of(jj * 4 * DH, 4 * DH), 4 * DH)], wq_buf.at[jj], sem_q.at[jj])

    LNG = 4
    d_c.start()
    d_wma.start()
    for b in range(LNG):
        d_x(b).start()

    d_c.wait()
    cf = c_buf[...].astype(F32)
    sc = _rb(cf * _sigmoid_b(cf))
    sc8 = jnp.broadcast_to(sc, (8, D)).astype(BF16)
    d_wma.wait()
    for b in range(LNG, 2 * LNG):
        d_x(b).start()
    mod_a = _rb(_dot(sc8, wma_buf[...]))
    sa = mod_a[0:1, 0:D]
    ca1 = _rb(1.0 + mod_a[0:1, D:2 * D])

    def ln1_body(g, carry):
        @pl.when(g == 0)
        def _():
            for b in range(2 * LNG, 3 * LNG):
                d_x(b).start()

        @pl.when(g == 1)
        def _():
            for b in range(3 * LNG, 4 * LNG):
                d_x(b).start()
            d_q(0).start()

        @pl.when(g == 2)
        def _():
            d_k(0).start()

        @pl.when(g == 3)
        def _():
            d_v(0).start()

        for t in range(LNG):
            d_x(g * LNG + t).wait()
        for t in range(LNG):
            b = g * LNG + t
            xf = x_buf[b].astype(F32)
            ln = _ln_t(xf).T
            hv = _rb(_rb(ln * ca1) + sa).astype(BF16)
            rows = pl.ds(pl.multiple_of(b * TB, TB), TB)
            for p in range(NP - 1):
                h_buf[p, rows, :] = hv[:, p * 128:(p + 1) * 128]
            h_buf[NP - 1, rows, :] = jnp.concatenate(
                [hv[:, (NP - 1) * 128:], jnp.zeros((TB, NP * 128 - D), BF16)], axis=1)
        return carry

    lax.fori_loop(0, NTB // LNG, ln1_body, 0)

    q_scale = np.float32(DH ** -0.5 * math.log2(math.e))
    NPAIR = HKV // 2
    HALF = S // 2

    def att_body(it, carry):
        jj = it // 2
        hf = it % 2

        @pl.when(hf == 0)
        def _():
            d_q(jj).wait()
            d_k(jj).wait()
            d_v(jj).wait()

        for b in range(HALF // R_ATT):
            rows = pl.ds(pl.multiple_of(hf * HALF + b * R_ATT, R_ATT), R_ATT)
            rows2 = pl.ds(pl.multiple_of((hf * HALF + b * R_ATT) // 2, R_ATT // 2), R_ATT // 2)
            hm = jnp.concatenate([as_bf16(h32[p, rows2, :]) for p in range(NP - 1)], axis=1)
            ht = as_bf16(h32[NP - 1, rows2, :])[:, :D - (NP - 1) * 128]
            wqv = wq_buf[jj]
            qf = _dot(hm, wqv[:(NP - 1) * 128, :]) + _dot(ht, wqv[(NP - 1) * 128:, :])
            q4 = (qf * q_scale).astype(BF16)
            for hh in range(4):
                j = 2 * jj + hh // 2
                q = q4[:, hh * DH:(hh + 1) * DH]
                s = _dot(q, as_bf16(k32[j]), NT_DIMS)
                m = jnp.max(s, axis=-1, keepdims=True)
                p = jnp.exp2(s - m)
                l = jnp.sum(p, axis=-1, keepdims=True)
                o = _dot(p.astype(BF16), as_bf16(v32[j]))
                o_buf[4 * jj + hh, rows, :] = (o * pltpu.reciprocal(l, approx=True)).astype(BF16)

        @pl.when(jnp.logical_and(hf == 0, jj + 1 < NPAIR))
        def _():
            d_q(jj + 1).start()
            d_k(jj + 1).start()
            d_v(jj + 1).start()

        pl.when(it == 1)(d_wmb.start)
        pl.when(it == 1)(d_wr.start)
        pl.when(it == 3)(d_wo.start)
        pl.when(it == 5)(d_wg.start)
        pl.when(it == 7)(d_wu.start)
        pl.when(it == 9)(d_wd.start)
        return carry

    lax.fori_loop(0, 2 * NPAIR, att_body, 0)

    d_wmb.wait()
    mod_b = _rb(_dot(sc8, wmb_buf[...]))
    gb = mod_b[0:1, 3 * D:4 * D]
    ga_c = _col(mod_b[0:1, 0:D])
    sb_c = _col(mod_b[0:1, D:2 * D])
    cb1_c = _col(_rb(1.0 + mod_b[0:1, 2 * D:3 * D]))
    gb_c = _col(gb)
    d_wr.wait()
    wr_c = _col(wr_buf[...].astype(F32).reshape(1, D))
    d_wo.wait()

    lane_id = lax.broadcasted_iota(jnp.int32, (1, TB), 1)

    def out_proj(b):
        toks = pl.ds(pl.multiple_of(b * TB, TB), TB)
        tok2 = pl.ds(pl.multiple_of(b * (TB // 2), TB // 2), TB // 2)
        o_cat = jnp.concatenate([as_bf16(o32[h, tok2, :]) for h in range(HQ)], axis=1)
        wo_t = jnp.concatenate([as_bf16(wo32[h]) for h in range(HQ)], axis=1)
        return _dot(wo_t, o_cat, NT_DIMS)

    def finish(b, attn):
        toks = pl.ds(pl.multiple_of(b * TB, TB), TB)
        x1 = _rb(x_buf[b].astype(F32) + ga_c * attn)
        h2 = _rb(_rb(_ln_t(x1) * cb1_c) + sb_c)
        r = _rb(jnp.sum(h2 * wr_c, axis=0, keepdims=True))
        key_buf[pl.ds(b, 1), :] = _sort_key(r, b * TB + lane_id)
        hb = h2 + h2 * 0.0
        out_buf[b] = (x1 + _rb(gb_c * hb)).astype(BF16)
        x1_buf[toks, :] = x1.T
        h2_buf[toks, :] = h2.T
        d_out(b).start()

    att_buf[...] = out_proj(0)

    def op_body(i, carry):
        prev = att_buf[...]
        for u in range(OP_UNROLL):
            b = 1 + i * OP_UNROLL + u
            cur = out_proj(b)
            finish(b - 1, prev)
            prev = cur
        att_buf[...] = prev
        return carry

    lax.fori_loop(0, (NTB - 1) // OP_UNROLL, op_body, 0)
    finish(NTB - 1, att_buf[...])

    key = key_buf[...]
    row8 = lax.broadcasted_iota(jnp.int32, (TOPK, 128), 0)
    sel = jnp.zeros((TOPK, 128), F32)
    for t in range(TOPK):
        m = jnp.max(jnp.max(key, axis=0, keepdims=True), axis=1, keepdims=True)
        sel = jnp.where(row8 == t, m, sel)
        key = jnp.where(key == m, 0.0, key)
    kb = lax.bitcast_convert_type(sel, jnp.int32) - KEY_BIAS
    idx_v = jnp.clip((S - 1) - (kb & (S - 1)), 0, S - 1)
    srt = lax.shift_right_logical(kb, 11)
    u16 = jnp.where(srt >= 0x8000, srt & 0x7FFF, 0xFFFF - srt)
    r_sel = lax.bitcast_convert_type(lax.shift_left(u16, 16), F32)[:, 0:1]
    for t in range(TOPK):
        idx_smem[t] = idx_v[t, 0]

    for t in range(TOPK):
        xs_buf[pl.ds(t, 1), :] = h2_buf[pl.ds(idx_smem[t], 1), :]
        xs_buf[pl.ds(TOPK + t, 1), :] = x1_buf[pl.ds(idx_smem[t], 1), :]
    xs = xs_buf[0:TOPK, :]
    xs_b = xs.astype(BF16)

    d_wg.wait()
    d_wu.wait()
    g = _rb(_dot(xs_b, wg_buf[...]))
    u = _rb(_dot(xs_b, wu_buf[...]))
    act = _rb(_rb(g * _sigmoid_b(g)) * u).astype(BF16)
    d_wd.wait()
    y = _rb(_dot(act, wd_buf[...], NT_DIMS))
    y = _rb(y * _sigmoid_b(r_sel))
    hb_sel = _rb(xs + _rb(_rb(xs * 0.0) + y))
    new = xs_buf[TOPK:2 * TOPK, :] + _rb(gb * hb_sel)
    new_t = jnp.concatenate([new, jnp.zeros((128 - TOPK, D), F32)], axis=0).T
    new_w = pltpu.bitcast(new_t.astype(BF16), jnp.int32)

    lane = lax.broadcasted_iota(jnp.int32, (D // 2, 128), 1)
    blk = [idx_smem[t] // TB for t in range(TOPK)]
    for b in range(NTB):
        d_out(b).wait()
    for t in range(TOPK):
        ln_t = idx_smem[t] % TB
        rolled = pltpu.roll(new_w, (ln_t + (TB - t)) % TB, axis=1)
        cur = pltpu.bitcast(out_buf[blk[t]], jnp.int32)
        out_buf[blk[t]] = pltpu.bitcast(jnp.where(lane == ln_t, rolled, cur), BF16)

    def d_patch(t):
        return cp(out_buf.at[blk[t]], out_hbm.at[:, pl.ds(pl.multiple_of(blk[t] * TB, TB), TB)], sem_patch.at[t])

    first = []
    for t in range(TOPK):
        f = blk[t] >= 0
        for t2 in range(t):
            f = jnp.logical_and(f, blk[t] != blk[t2])
        first.append(f)
    for t in range(TOPK):
        pl.when(first[t])(lambda t=t: d_patch(t).start())
    for t in range(TOPK):
        pl.when(first[t])(lambda t=t: d_patch(t).wait())


@jax.jit
def pallas_adaLN_cond__gqa_block_cached__moe_arch_mod__prompt_kernel(
    A_x, A_k_cache, A_v_cache, A_wq, A_wo, B_x, B_w_r, B_w_gate, B_w_up, B_w_down, c, w_mod,
):
    del B_x
    xt = A_x.reshape(S, D).T
    k = A_k_cache.reshape(HKV, S, DH)
    v = A_v_cache.reshape(HKV, S, DH)
    hbm = pl.BlockSpec(memory_space=pl.ANY)
    out = pl.pallas_call(
        _kernel,
        in_specs=[hbm] * 11,
        out_specs=hbm,
        out_shape=jax.ShapeDtypeStruct((D, S), BF16),
        scratch_shapes=[
            pltpu.VMEM((NTB, D, TB), BF16),
            pltpu.VMEM((NP, S, 128), BF16),
            pltpu.VMEM((HKV, S, DH), BF16),
            pltpu.VMEM((HKV, S, DH), BF16),
            pltpu.VMEM((HKV // 2, D, 4 * DH), BF16),
            pltpu.VMEM((HQ, D, DH), BF16),
            pltpu.VMEM((D,), BF16),
            pltpu.VMEM((D, F), BF16),
            pltpu.VMEM((D, F), BF16),
            pltpu.VMEM((D, F), BF16),
            pltpu.VMEM((1, D), BF16),
            pltpu.VMEM((D, 2 * D), BF16),
            pltpu.VMEM((D, 4 * D), BF16),
            pltpu.VMEM((HQ, S, DH), BF16),
            pltpu.VMEM((S, D), F32),
            pltpu.VMEM((S, D), F32),
            pltpu.VMEM((NTB, D, TB), BF16),
            pltpu.VMEM((NTB, TB), F32),
            pltpu.VMEM((D, TB), F32),
            pltpu.VMEM((2 * TOPK, D), F32),
            pltpu.SMEM((TOPK,), jnp.int32),
            pltpu.SemaphoreType.DMA((9,)),
            pltpu.SemaphoreType.DMA((HKV // 2,)),
            pltpu.SemaphoreType.DMA((HKV // 2,)),
            pltpu.SemaphoreType.DMA((HKV // 2,)),
            pltpu.SemaphoreType.DMA((NTB,)),
            pltpu.SemaphoreType.DMA((NTB,)),
            pltpu.SemaphoreType.DMA((TOPK,)),
        ],
        compiler_params=pltpu.CompilerParams(vmem_limit_bytes=120 * 1024 * 1024, disable_bounds_checks=True),
    )(xt, k, v, A_wq, A_wo.T, B_w_r, B_w_gate, B_w_up, B_w_down.T, c, w_mod)
    return out.T.reshape(1, S, D)
```

```python
import functools
import math

import jax
import jax.numpy as jnp
import numpy as np
from jax import lax
from jax.experimental import pallas as pl
from jax.experimental.pallas import tpu as pltpu

S = 2048
D = 576
HQ = 32
HKV = 16
DH = 128
F = 4608
TOPK = 8
EPS = 1e-5
TB = 128
NTB = S // TB
NP = D // 128
DM = NP * 128

RBLK = [288] + [272] * 14
R_ATT = 256
R_LN = 256

F32 = jnp.float32
BF16 = jnp.bfloat16
NT_DIMS = (((1,), (1,)), ((), ()))
NN_DIMS = (((1,), (0,)), ((), ()))


def _rb(v):
    return v.astype(BF16).astype(F32)


def _dot(a, b, dims=NN_DIMS):
    return lax.dot_general(a, b, dims, preferred_element_type=F32)


def _sigmoid_b(g):
    return _rb(1.0 / _rb(1.0 + _rb(jnp.exp(-g))))


def _ln_t(xf):
    inv_d = np.float32(1.0 / D)
    m32 = jnp.sum(xf, axis=0, keepdims=True) * inv_d
    cen = xf - m32
    v = _rb(jnp.sum(cen * cen, axis=0, keepdims=True) * inv_d)
    eps_b = np.float32(np.float32(EPS).astype(jnp.bfloat16))
    den = _rb(jnp.sqrt(_rb(v + eps_b)))
    inv = 1.0 / den
    return _rb(_rb(xf - _rb(m32)) * inv)


def _ln1_t(xf):
    inv_d = np.float32(1.0 / D)
    m32 = jnp.sum(xf, axis=0, keepdims=True) * inv_d
    cen = xf - m32
    v = jnp.sum(cen * cen, axis=0, keepdims=True) * inv_d
    return cen * lax.rsqrt(v + np.float32(EPS))


def _col(row):
    return jnp.broadcast_to(row, (128, D)).T


KEY_BIAS = 0x20000000


def _sort_key(r, tok):
    bits = lax.bitcast_convert_type(r, jnp.int32)
    u = lax.shift_right_logical(bits, 16)
    u = jnp.where(u == 0x8000, 0, u)
    srt = jnp.where(u >= 0x8000, 0xFFFF - u, u | 0x8000)
    srt = jnp.where(r != r, 0, srt)
    key = lax.shift_left(srt, 11) | (S - 1 - tok)
    return lax.bitcast_convert_type(key + KEY_BIAS, F32)


def _kernel(xt_hbm, k_hbm, v_hbm, wq_hbm, wot_hbm, wr_hbm, wg_hbm, wu_hbm, wdt_hbm, c_hbm, wmod_hbm,
            out_hbm,
            x_buf, h_buf, ht_buf, q_buf, k_buf, v_buf, wq_buf, wo_buf, wr_buf, wg_buf, wu_buf, wd_buf, c_buf,
            wma_buf, wmb_buf, o2_buf, xh_buf, out_buf, key_buf, att_buf, acc_buf, x1t_buf, h2t_buf, col_buf, xs_buf, idx_smem,
            sem_misc, sem_k, sem_v, sem_q, sem_x, sem_out, sem_patch):
    k32 = k_buf.bitcast(jnp.int32)
    v32 = v_buf.bitcast(jnp.int32)
    o32 = o2_buf.bitcast(jnp.int32)
    h32 = h_buf.bitcast(jnp.int32)
    ht32 = ht_buf.bitcast(jnp.int32)
    q32 = q_buf.bitcast(jnp.int32)
    wo32 = wo_buf.bitcast(jnp.int32)

    def as_bf16(v):
        return pltpu.bitcast(v, BF16)

    def cp(src, dst, sem):
        return pltpu.make_async_copy(src, dst, sem)

    d_c = cp(c_hbm, c_buf, sem_misc.at[0])
    d_wma = cp(wmod_hbm.at[:, pl.ds(0, 2 * D)], wma_buf, sem_misc.at[1])
    d_wmb = cp(wmod_hbm.at[:, pl.ds(2 * D, 4 * D)], wmb_buf, sem_misc.at[3])

    class _Group:
        def __init__(self, copies):
            self.copies = copies

        def start(self):
            for c in self.copies:
                c.start()

        def wait(self):
            for c in self.copies:
                c.wait()

    d_wo = _Group([cp(wot_hbm.at[:, pl.ds(h * DH, DH)], wo_buf.at[h], sem_misc.at[4]) for h in range(HQ)])
    d_wr = cp(wr_hbm, wr_buf, sem_misc.at[5])
    d_wg = cp(wg_hbm, wg_buf, sem_misc.at[6])
    d_wu = cp(wu_hbm, wu_buf, sem_misc.at[7])
    d_wd = cp(wdt_hbm, wd_buf, sem_misc.at[8])

    def d_x(b):
        return cp(xt_hbm.at[:, pl.ds(pl.multiple_of(b * TB, TB), TB)], x_buf.at[b], sem_x.at[b])

    def d_out(b):
        return cp(out_buf.at[b], out_hbm.at[:, pl.ds(pl.multiple_of(b * TB, TB), TB)], sem_out.at[b])

    def d_k(j):
        return cp(k_hbm.at[j], k_buf.at[j], sem_k.at[j])

    def d_v(j):
        return cp(v_hbm.at[j], v_buf.at[j], sem_v.at[j])

    def d_q(j):
        return cp(wq_hbm.at[:, pl.ds(pl.multiple_of(j * 2 * DH, 2 * DH), 2 * DH)], wq_buf.at[j], sem_q.at[j])

    LNG = 4
    d_c.start()
    d_wma.start()
    for b in range(LNG):
        d_x(b).start()

    d_c.wait()
    cf = c_buf[...].astype(F32)
    sc = _rb(cf * _sigmoid_b(cf))
    sc8 = jnp.broadcast_to(sc, (8, D)).astype(BF16)
    d_wma.wait()
    for b in range(LNG, 2 * LNG):
        d_x(b).start()
    mod_a = _rb(_dot(sc8, wma_buf[...]))
    col_buf[0] = _col(_rb(1.0 + mod_a[0:1, D:2 * D]))
    col_buf[1] = _col(mod_a[0:1, 0:D])

    def ln1_body(g, carry):
        @pl.when(g == 0)
        def _():
            for b in range(2 * LNG, 3 * LNG):
                d_x(b).start()

        @pl.when(g == 1)
        def _():
            for b in range(3 * LNG, 4 * LNG):
                d_x(b).start()
            d_q(0).start()

        @pl.when(g == 2)
        def _():
            d_k(0).start()

        @pl.when(g == 3)
        def _():
            d_v(0).start()

        for t in range(LNG):
            d_x(g * LNG + t).wait()
        tails = []
        for t in range(LNG):
            b = g * LNG + t
            xf = x_buf[b].astype(F32)
            ht = _ln1_t(xf) * col_buf[0] + col_buf[1]
            hv = ht[:DM, :].T.astype(BF16)
            rows = pl.ds(pl.multiple_of(b * TB, TB), TB)
            for p in range(NP):
                h_buf[p, rows, :] = hv[:, p * 128:(p + 1) * 128]
            tails.append(ht[DM:, :])
        for t in range(2):
            rows = pl.ds(pl.multiple_of((2 * g + t) * TB, TB), TB)
            ht_buf[rows, :] = jnp.concatenate([tails[t], tails[t + 2]], axis=0).T.astype(BF16)
        return carry

    lax.fori_loop(0, NTB // LNG, ln1_body, 0)

    q_scale = np.float32(DH ** -0.5 * math.log2(math.e))

    def prefetch(j):
        d_q(j).start()
        d_k(j).start()
        d_v(j).start()

    def att_body(j, carry):
        d_q(j).wait()
        pl.when(j > 0)(lambda: d_k(j).wait())
        d_v(j).wait()

        wqv = wq_buf[j]
        w_tail = wqv[DM:, :]
        zero = jnp.zeros_like(w_tail)
        w2 = jnp.concatenate([jnp.concatenate([w_tail, zero], axis=1),
                              jnp.concatenate([zero, w_tail], axis=1)], axis=0)
        RQ = 256
        for g in range(S // (2 * RQ)):
            ht = as_bf16(ht32[pl.ds(g * (RQ // 2), RQ // 2), :])
            q_tail = _dot(ht, w2)
            for u in range(2):
                b = 2 * g + u
                rows = pl.ds(b * RQ, RQ)
                rows2 = pl.ds(b * (RQ // 2), RQ // 2)
                hm = jnp.concatenate([as_bf16(h32[p, rows2, :]) for p in range(NP)], axis=1)
                qf = _dot(hm, wqv[:DM, :]) + q_tail[:, u * 2 * DH:(u + 1) * 2 * DH]
                q2 = (qf * q_scale).astype(BF16)
                q_buf[pl.ds(b * RQ, RQ), :] = q2[:, :DH]
                q_buf[pl.ds(S + b * RQ, RQ), :] = q2[:, DH:]
        r0 = 0
        for rsz in RBLK:
            rows = pl.ds(r0, rsz)
            q = as_bf16(q32[pl.ds(r0 // 2, rsz // 2), :])
            s = _dot(q, as_bf16(k32[j]), NT_DIMS)
            m = jnp.max(s, axis=-1, keepdims=True)
            p = jnp.exp2(s - m)
            l = jnp.sum(p, axis=-1, keepdims=True)
            o = _dot(p.astype(BF16), as_bf16(v32[j]))
            o2_buf[j, rows, :] = (o * pltpu.reciprocal(l, approx=True)).astype(BF16)
            r0 += rsz

        pl.when(j + 2 < HKV)(lambda: prefetch(j + 2))
        pl.when(j == 1)(d_wmb.start)
        pl.when(j == 1)(d_wr.start)
        pl.when(j == 3)(d_wo.start)
        pl.when(j == 5)(d_wg.start)
        pl.when(j == 7)(d_wu.start)
        pl.when(j == 9)(d_wd.start)
        return carry

    d_k(0).wait()
    prefetch(1)
    lax.fori_loop(0, HKV, att_body, 0)

    d_wmb.wait()
    d_wr.wait()
    d_wo.wait()
    mod_b = _rb(_dot(sc8, wmb_buf[...]))
    gb = mod_b[0:1, 3 * D:4 * D]
    col_buf[0] = _col(mod_b[0:1, 0:D])
    col_buf[1] = _col(mod_b[0:1, D:2 * D])
    col_buf[2] = _col(_rb(1.0 + mod_b[0:1, 2 * D:3 * D]))
    col_buf[3] = _col(gb)
    col_buf[4] = _col(wr_buf[...].astype(F32).reshape(1, D))

    lane_id = lax.broadcasted_iota(jnp.int32, (1, TB), 1)

    NG = 8
    HG = HQ // NG
    CH = 8
    NC = D // CH
    inv_d = np.float32(1.0 / D)
    eps_b = np.float32(np.float32(EPS).astype(jnp.bfloat16))

    def part_of(b, g):
        def tok2_of(h):
            return pl.ds(pl.multiple_of((h % 2) * (S // 2) + b * (TB // 2), TB // 2), TB // 2)
        heads = range(g * HG, (g + 1) * HG)
        o_cat = jnp.concatenate([as_bf16(o32[h // 2, tok2_of(h), :]) for h in heads], axis=1)
        wo_t = jnp.concatenate([as_bf16(wo32[h]) for h in heads], axis=1)
        return _dot(wo_t, o_cat, NT_DIMS)

    def accumulate(dst, src, part):
        for c in range(NC):
            r = slice(c * CH, (c + 1) * CH)
            dst[r, :] = part[r, :] if src is None else src[r, :] + part[r, :]

    def stage_a(p, att, x1_dst):
        acc = None
        for c in range(NC):
            r = slice(c * CH, (c + 1) * CH)
            c16 = slice((c // 2) * 16, (c // 2) * 16 + 16)
            xv = x_buf[p, c16, :].astype(F32)[(c % 2) * 8:(c % 2) * 8 + 8, :]
            x1 = _rb(xv + col_buf[0, r, :] * att[r, :])
            x1_dst[r, :] = x1
            acc = x1 if acc is None else acc + x1
        return jnp.sum(acc, axis=0, keepdims=True) * inv_d

    def stage_b(x1_src, m32):
        acc = None
        for c in range(NC):
            r = slice(c * CH, (c + 1) * CH)
            cen = x1_src[r, :] - m32
            acc = cen * cen if acc is None else acc + cen * cen
        v = _rb(jnp.sum(acc, axis=0, keepdims=True) * inv_d)
        return 1.0 / _rb(jnp.sqrt(_rb(v + eps_b)))

    def stage_c(p, x1_src, m32, inv, h_dst):
        mb = _rb(m32)
        acc = None
        for c2 in range(NC // 2):
            outs = []
            for c in (2 * c2, 2 * c2 + 1):
                r = slice(c * CH, (c + 1) * CH)
                x1 = x1_src[r, :]
                h2 = _rb(_rb(_rb(_rb(x1 - mb) * inv) * col_buf[2, r, :]) + col_buf[1, r, :])
                t = h2 * col_buf[4, r, :]
                acc = t if acc is None else acc + t
                hb = h2 + h2 * 0.0
                outs.append(x1 + _rb(col_buf[3, r, :] * hb))
                h_dst[r, :] = (lax.bitcast_convert_type(h2, jnp.int32)
                               | lax.shift_right_logical(lax.bitcast_convert_type(x1, jnp.int32), 16))
            out_buf[p, 16 * c2:16 * c2 + 16, :] = jnp.concatenate(outs, axis=0).astype(BF16)
        r_tok = _rb(jnp.sum(acc, axis=0, keepdims=True))
        key_buf[pl.ds(p, 1), :] = _sort_key(r_tok, p * TB + lane_id)

    def stage_d(p, h_src):
        xh_buf[pl.ds(pl.multiple_of(p * TB, TB), TB), :] = h_src[...].T

    def op_block(b, carry):
        p = b - 1
        z = b & 1
        bA, bB, bH = acc_buf.at[z], x1t_buf.at[z], h2t_buf.at[z]
        bX, bXn = att_buf.at[z], att_buf.at[1 - z]
        accumulate(bA, None, part_of(b, 0))
        m32 = stage_a(p, bX, bB)
        accumulate(bA, bA, part_of(b, 1))
        accumulate(bX, bA, part_of(b, 2))
        inv = stage_b(bB, m32)
        accumulate(bX, bX, part_of(b, 3))
        stage_c(p, bB, m32, inv, bH)
        accumulate(bB, bX, part_of(b, 4))
        accumulate(bB, bB, part_of(b, 5))
        accumulate(bB, bB, part_of(b, 6))
        stage_d(p, bH)
        accumulate(bXn, bB, part_of(b, 7))
        d_out(p).start()
        return carry

    accumulate(acc_buf.at[0], None, part_of(0, 0))
    for g in range(1, NG - 1):
        accumulate(acc_buf.at[0], acc_buf.at[0], part_of(0, g))
    accumulate(att_buf.at[1], acc_buf.at[0], part_of(0, NG - 1))
    lax.fori_loop(1, NTB, op_block, 0)
    zl = NTB & 1
    m32 = stage_a(NTB - 1, att_buf.at[zl], x1t_buf.at[zl])
    inv = stage_b(x1t_buf.at[zl], m32)
    stage_c(NTB - 1, x1t_buf.at[zl], m32, inv, h2t_buf.at[zl])
    d_out(NTB - 1).start()
    stage_d(NTB - 1, h2t_buf.at[zl])

    key = key_buf[...]
    row8 = lax.broadcasted_iota(jnp.int32, (TOPK, 128), 0)
    sel = jnp.zeros((TOPK, 128), F32)
    for t in range(TOPK):
        m = jnp.max(jnp.max(key, axis=0, keepdims=True), axis=1, keepdims=True)
        sel = jnp.where(row8 == t, m, sel)
        key = jnp.where(key == m, 0.0, key)
    kb = lax.bitcast_convert_type(sel, jnp.int32) - KEY_BIAS
    idx_v = jnp.clip((S - 1) - (kb & (S - 1)), 0, S - 1)
    srt = lax.shift_right_logical(kb, 11)
    u16 = jnp.where(srt >= 0x8000, srt & 0x7FFF, 0xFFFF - srt)
    r_sel = lax.bitcast_convert_type(lax.shift_left(u16, 16), F32)[:, 0:1]
    for t in range(TOPK):
        idx_smem[t] = idx_v[t, 0]

    for t in range(TOPK):
        xs_buf[pl.ds(t, 1), :] = xh_buf[pl.ds(idx_smem[t], 1), :]
    xw = xs_buf[...]
    xs = lax.bitcast_convert_type(xw & jnp.int32(-65536), F32)
    x1s = lax.bitcast_convert_type(lax.shift_left(xw, 16), F32)
    xs_b = xs.astype(BF16)

    d_wg.wait()
    d_wu.wait()
    g = _rb(_dot(xs_b, wg_buf[...]))
    u = _rb(_dot(xs_b, wu_buf[...]))
    act = _rb(_rb(g * _sigmoid_b(g)) * u).astype(BF16)
    d_wd.wait()
    y = _rb(_dot(act, wd_buf[...], NT_DIMS))
    y = _rb(y * _sigmoid_b(r_sel))
    hb_sel = _rb(xs + _rb(_rb(xs * 0.0) + y))
    new = x1s + _rb(gb * hb_sel)
    new_t = jnp.concatenate([new, jnp.zeros((128 - TOPK, D), F32)], axis=0).T
    new_w = pltpu.bitcast(new_t.astype(BF16), jnp.int32)

    lane = lax.broadcasted_iota(jnp.int32, (D // 2, 128), 1)
    blk = [idx_smem[t] // TB for t in range(TOPK)]
    for b in range(NTB):
        d_out(b).wait()
    for t in range(TOPK):
        ln_t = idx_smem[t] % TB
        rolled = pltpu.roll(new_w, (ln_t + (TB - t)) % TB, axis=1)
        cur = pltpu.bitcast(out_buf[blk[t]], jnp.int32)
        out_buf[blk[t]] = pltpu.bitcast(jnp.where(lane == ln_t, rolled, cur), BF16)

    def d_patch(t):
        return cp(out_buf.at[blk[t]], out_hbm.at[:, pl.ds(pl.multiple_of(blk[t] * TB, TB), TB)], sem_patch.at[t])

    first = []
    for t in range(TOPK):
        f = blk[t] >= 0
        for t2 in range(t):
            f = jnp.logical_and(f, blk[t] != blk[t2])
        first.append(f)
    for t in range(TOPK):
        pl.when(first[t])(lambda t=t: d_patch(t).start())
    for t in range(TOPK):
        pl.when(first[t])(lambda t=t: d_patch(t).wait())


@jax.jit
def pallas_adaLN_cond__gqa_block_cached__moe_arch_mod__prompt_kernel(
    A_x, A_k_cache, A_v_cache, A_wq, A_wo, B_x, B_w_r, B_w_gate, B_w_up, B_w_down, c, w_mod,
):
    del B_x
    xt = A_x.reshape(S, D).T
    k = A_k_cache.reshape(HKV, S, DH)
    v = A_v_cache.reshape(HKV, S, DH)
    hbm = pl.BlockSpec(memory_space=pl.ANY)
    out = pl.pallas_call(
        _kernel,
        in_specs=[hbm] * 11,
        out_specs=hbm,
        out_shape=jax.ShapeDtypeStruct((D, S), BF16),
        scratch_shapes=[
            pltpu.VMEM((NTB, D, TB), BF16),
            pltpu.VMEM((NP, S, 128), BF16),
            pltpu.VMEM((S // 2, 128), BF16),
            pltpu.VMEM((2 * S, DH), BF16),
            pltpu.VMEM((HKV, S, DH), BF16),
            pltpu.VMEM((HKV, S, DH), BF16),
            pltpu.VMEM((HKV, D, 2 * DH), BF16),
            pltpu.VMEM((HQ, D, DH), BF16),
            pltpu.VMEM((D,), BF16),
            pltpu.VMEM((D, F), BF16),
            pltpu.VMEM((D, F), BF16),
            pltpu.VMEM((D, F), BF16),
            pltpu.VMEM((1, D), BF16),
            pltpu.VMEM((D, 2 * D), BF16),
            pltpu.VMEM((D, 4 * D), BF16),
            pltpu.VMEM((HKV, 2 * S, DH), BF16),
            pltpu.VMEM((S, D), jnp.int32),
            pltpu.VMEM((NTB, D, TB), BF16),
            pltpu.VMEM((NTB, TB), F32),
            pltpu.VMEM((2, D, TB), F32),
            pltpu.VMEM((2, D, TB), F32),
            pltpu.VMEM((2, D, TB), F32),
            pltpu.VMEM((2, D, TB), jnp.int32),
            pltpu.VMEM((5, D, TB), F32),
            pltpu.VMEM((TOPK, D), jnp.int32),
            pltpu.SMEM((TOPK,), jnp.int32),
            pltpu.SemaphoreType.DMA((9,)),
            pltpu.SemaphoreType.DMA((HKV,)),
            pltpu.SemaphoreType.DMA((HKV,)),
            pltpu.SemaphoreType.DMA((HKV,)),
            pltpu.SemaphoreType.DMA((NTB,)),
            pltpu.SemaphoreType.DMA((NTB,)),
            pltpu.SemaphoreType.DMA((TOPK,)),
        ],
        compiler_params=pltpu.CompilerParams(vmem_limit_bytes=120 * 1024 * 1024, disable_bounds_checks=True),
    )(xt, k, v, A_wq, A_wo.T, B_w_r, B_w_gate, B_w_up, B_w_down.T, c, w_mod)
    return out.T.reshape(1, S, D)
```

```python
import functools
import math

import jax
import jax.numpy as jnp
import numpy as np
from jax import lax
from jax.experimental import pallas as pl
from jax.experimental.pallas import tpu as pltpu

S = 2048
D = 576
HQ = 32
HKV = 16
DH = 128
F = 4608
TOPK = 8
EPS = 1e-5
TB = 128
NTB = S // TB
OB = 256
NP = D // 128
DM = NP * 128

RBLK = [288] + [272] * 14
R_ATT = 256
R_LN = 256

F32 = jnp.float32
BF16 = jnp.bfloat16
NT_DIMS = (((1,), (1,)), ((), ()))
NN_DIMS = (((1,), (0,)), ((), ()))


def _rb(v):
    return v.astype(BF16).astype(F32)


def _dot(a, b, dims=NN_DIMS):
    return lax.dot_general(a, b, dims, preferred_element_type=F32)


def _sigmoid_b(g):
    return _rb(1.0 / _rb(1.0 + _rb(jnp.exp(-g))))


def _ln_t(xf):
    inv_d = np.float32(1.0 / D)
    m32 = jnp.sum(xf, axis=0, keepdims=True) * inv_d
    cen = xf - m32
    v = _rb(jnp.sum(cen * cen, axis=0, keepdims=True) * inv_d)
    eps_b = np.float32(np.float32(EPS).astype(jnp.bfloat16))
    den = _rb(jnp.sqrt(_rb(v + eps_b)))
    inv = 1.0 / den
    return _rb(_rb(xf - _rb(m32)) * inv)


def _ln1_t(xf):
    inv_d = np.float32(1.0 / D)
    m32 = jnp.sum(xf, axis=0, keepdims=True) * inv_d
    cen = xf - m32
    v = jnp.sum(cen * cen, axis=0, keepdims=True) * inv_d
    return cen * lax.rsqrt(v + np.float32(EPS))


def _col(row):
    return jnp.broadcast_to(row, (128, D)).T


KEY_BIAS = 0x20000000


def _sort_key(r, tok):
    bits = lax.bitcast_convert_type(r, jnp.int32)
    u = lax.shift_right_logical(bits, 16)
    u = jnp.where(u == 0x8000, 0, u)
    srt = jnp.where(u >= 0x8000, 0xFFFF - u, u | 0x8000)
    srt = jnp.where(r != r, 0, srt)
    key = lax.shift_left(srt, 11) | (S - 1 - tok)
    return lax.bitcast_convert_type(key + KEY_BIAS, F32)


def _kernel(xt_hbm, k_hbm, v_hbm, wq_hbm, wot_hbm, wr_hbm, wg_hbm, wu_hbm, wdt_hbm, c_hbm, wmod_hbm,
            out_hbm,
            x_buf, h_buf, ht_buf, q_buf, k_buf, v_buf, wq_buf, wo_buf, wr_buf, wg_buf, wu_buf, wd_buf, wdn_buf, c_buf,
            wma_buf, wmb_buf, o2_buf, xh_buf, out_buf, key_buf, top_buf, att_buf, acc_buf, x1t_buf, h2t_buf, col_buf, gb_buf, xs_buf, idx_smem, top_smem,
            sem_misc, sem_k, sem_v, sem_q, sem_x, sem_out, sem_patch):
    k32 = k_buf.bitcast(jnp.int32)
    v32 = v_buf.bitcast(jnp.int32)
    o32 = o2_buf.bitcast(jnp.int32)
    h32 = h_buf.bitcast(jnp.int32)
    ht32 = ht_buf.bitcast(jnp.int32)
    q32 = q_buf.bitcast(jnp.int32)
    wo32 = wo_buf.bitcast(jnp.int32)
    out32 = out_buf.bitcast(jnp.int32)

    def as_bf16(v):
        return pltpu.bitcast(v, BF16)

    def cp(src, dst, sem):
        return pltpu.make_async_copy(src, dst, sem)

    d_c = cp(c_hbm, c_buf, sem_misc.at[0])
    d_wma = cp(wmod_hbm.at[:, pl.ds(0, 2 * D)], wma_buf, sem_misc.at[1])
    d_wmb = cp(wmod_hbm.at[:, pl.ds(2 * D, 4 * D)], wmb_buf, sem_misc.at[3])

    class _Group:
        def __init__(self, copies):
            self.copies = copies

        def start(self):
            for c in self.copies:
                c.start()

        def wait(self):
            for c in self.copies:
                c.wait()

    d_wo = _Group([cp(wot_hbm.at[:, pl.ds(h * DH, DH)], wo_buf.at[h], sem_misc.at[4]) for h in range(HQ)])
    d_wr = cp(wr_hbm, wr_buf, sem_misc.at[5])
    d_wg = cp(wg_hbm, wg_buf, sem_misc.at[6])
    d_wu = cp(wu_hbm, wu_buf, sem_misc.at[7])
    d_wd = cp(wdt_hbm, wd_buf, sem_misc.at[8])

    def d_x(b):
        return cp(xt_hbm.at[:, pl.ds(pl.multiple_of(b * TB, TB), TB)], x_buf.at[b], sem_x.at[b])

    def d_out(b):
        return cp(out_buf.at[b], out_hbm.at[:, pl.ds(pl.multiple_of(b * TB, TB), TB)], sem_out.at[b])

    def d_k(j):
        return cp(k_hbm.at[j], k_buf.at[j], sem_k.at[j])

    def d_v(j):
        return cp(v_hbm.at[j], v_buf.at[j], sem_v.at[j])

    def d_q(j):
        return cp(wq_hbm.at[:, pl.ds(pl.multiple_of(j * 2 * DH, 2 * DH), 2 * DH)], wq_buf.at[j], sem_q.at[j])

    LNG = 4
    d_c.start()
    d_wma.start()
    for b in range(NTB):
        d_x(b).start(priority=1)
    d_q(0).start(priority=1)
    d_k(0).start(priority=1)
    d_v(0).start(priority=1)

    d_c.wait()
    cf = c_buf[...].astype(F32)
    sc = _rb(cf * _sigmoid_b(cf))
    sc8 = jnp.broadcast_to(sc, (8, D)).astype(BF16)
    d_wma.wait()
    mod_a = _rb(_dot(sc8, wma_buf[...]))
    col_buf[0] = _col(_rb(1.0 + mod_a[0:1, D:2 * D]))
    col_buf[1] = _col(mod_a[0:1, 0:D])

    def ln1_body(g, carry):
        for t in range(LNG):
            d_x(g * LNG + t).wait()
        tails = []
        for t in range(LNG):
            b = g * LNG + t
            xf = x_buf[b].astype(F32)
            ht = _ln1_t(xf) * col_buf[0] + col_buf[1]
            hv = ht[:DM, :].T.astype(BF16)
            rows = pl.ds(pl.multiple_of(b * TB, TB), TB)
            for p in range(NP):
                h_buf[p, rows, :] = hv[:, p * 128:(p + 1) * 128]
            tails.append(ht[DM:, :])
        for t in range(2):
            rows = pl.ds(pl.multiple_of((2 * g + t) * TB, TB), TB)
            ht_buf[rows, :] = jnp.concatenate([tails[t], tails[t + 2]], axis=0).T.astype(BF16)
        return carry

    lax.fori_loop(0, NTB // LNG, ln1_body, 0)

    q_scale = np.float32(DH ** -0.5 * math.log2(math.e))

    def prefetch(j):
        d_q(j).start(priority=1)
        d_k(j).start(priority=1)
        d_v(j).start(priority=1)

    def att_body(j, carry):
        d_q(j).wait()
        pl.when(j > 0)(lambda: d_k(j).wait())
        pl.when(j > 0)(lambda: d_v(j).wait())

        wqv = wq_buf[j]
        w_tail = wqv[DM:, :]
        zero = jnp.zeros_like(w_tail)
        w2 = jnp.concatenate([jnp.concatenate([w_tail, zero], axis=1),
                              jnp.concatenate([zero, w_tail], axis=1)], axis=0)
        RQ = 256
        for g in range(S // (2 * RQ)):
            ht = as_bf16(ht32[pl.ds(g * (RQ // 2), RQ // 2), :])
            q_tail = _dot(ht, w2)
            for u in range(2):
                b = 2 * g + u
                rows = pl.ds(b * RQ, RQ)
                rows2 = pl.ds(b * (RQ // 2), RQ // 2)
                hm = jnp.concatenate([as_bf16(h32[p, rows2, :]) for p in range(NP)], axis=1)
                qf = _dot(hm, wqv[:DM, :]) + q_tail[:, u * 2 * DH:(u + 1) * 2 * DH]
                q2 = (qf * q_scale).astype(BF16)
                q_buf[pl.ds(b * RQ, RQ), :] = q2[:, :DH]
                q_buf[pl.ds(S + b * RQ, RQ), :] = q2[:, DH:]
        r0 = 0
        for rsz in RBLK:
            rows = pl.ds(r0, rsz)
            q = as_bf16(q32[pl.ds(r0 // 2, rsz // 2), :])
            s = _dot(q, as_bf16(k32[j]), NT_DIMS)
            m = jnp.max(s, axis=-1, keepdims=True)
            p = jnp.exp2(s - m)
            l = jnp.sum(p, axis=-1, keepdims=True)
            o = _dot(p.astype(BF16), as_bf16(v32[j]))
            o2_buf[j, rows, :] = (o * pltpu.reciprocal(l, approx=True)).astype(BF16)
            r0 += rsz

        pl.when(j + 2 < HKV)(lambda: prefetch(j + 2))
        pl.when(j == 1)(d_wmb.start)
        pl.when(j == 1)(d_wr.start)
        pl.when(j == 3)(d_wo.start)
        pl.when(j == 5)(d_wg.start)
        pl.when(j == 7)(d_wu.start)
        pl.when(j == 9)(d_wd.start)
        return carry

    d_k(0).wait()
    d_v(0).wait()
    prefetch(1)
    lax.fori_loop(0, HKV, att_body, 0)

    d_wmb.wait()
    d_wr.wait()
    d_wo.wait()
    d_wd.wait()
    mod_b = _rb(_dot(sc8, wmb_buf[...]))
    gb = mod_b[0:1, 3 * D:4 * D]
    gb_buf[...] = gb
    col_buf[0] = _col(mod_b[0:1, 0:D])
    col_buf[1] = _col(mod_b[0:1, D:2 * D])
    col_buf[2] = _col(_rb(1.0 + mod_b[0:1, 2 * D:3 * D]))
    col_buf[3] = _col(gb)
    col_buf[4] = _col(wr_buf[...].astype(F32).reshape(1, D))

    lane_id = lax.broadcasted_iota(jnp.int32, (1, TB), 1)

    NG = 8
    HG = HQ // NG
    CH = 8
    NC = D // CH
    NLB = OB // TB
    NOB = S // OB
    inv_d = np.float32(1.0 / D)
    eps_b = np.float32(np.float32(EPS).astype(jnp.bfloat16))

    def lanes(t):
        return slice(t * TB, (t + 1) * TB)

    def part_of(b, g):
        def tok2_of(h):
            return pl.ds(pl.multiple_of((h % 2) * (S // 2) + b * (OB // 2), OB // 2), OB // 2)
        heads = range(g * HG, (g + 1) * HG)
        o_cat = jnp.concatenate([as_bf16(o32[h // 2, tok2_of(h), :]) for h in heads], axis=1)
        wo_t = jnp.concatenate([as_bf16(wo32[h]) for h in heads], axis=1)
        return _dot(wo_t, o_cat, NT_DIMS)

    def accumulate(dst, src, part):
        for c in range(NC):
            r = slice(c * CH, (c + 1) * CH)
            dst[r, :] = part[r, :] if src is None else src[r, :] + part[r, :]

    def stage_a(p, att, x1_dst):
        means = []
        for t in range(NLB):
            acc = None
            for c in range(NC):
                r = slice(c * CH, (c + 1) * CH)
                c16 = slice((c // 2) * 16, (c // 2) * 16 + 16)
                xv = x_buf[p * NLB + t, c16, :].astype(F32)[(c % 2) * 8:(c % 2) * 8 + 8, :]
                x1 = _rb(xv + col_buf[0, r, :] * att[r, lanes(t)])
                x1_dst[r, lanes(t)] = x1
                acc = x1 if acc is None else acc + x1
            means.append(jnp.sum(acc, axis=0, keepdims=True) * inv_d)
        return means

    def stage_b(x1_src, means):
        invs = []
        for t in range(NLB):
            acc = None
            for c in range(NC):
                r = slice(c * CH, (c + 1) * CH)
                cen = x1_src[r, lanes(t)] - means[t]
                acc = cen * cen if acc is None else acc + cen * cen
            v = _rb(jnp.sum(acc, axis=0, keepdims=True) * inv_d)
            invs.append(1.0 / _rb(jnp.sqrt(_rb(v + eps_b))))
        return invs

    def stage_c(p, x1_src, means, invs, h_dst):
        mb = [_rb(m) for m in means]
        acc = [None] * NLB
        for c2 in range(NC // 2):
            for t in range(NLB):
                outs = []
                for c in (2 * c2, 2 * c2 + 1):
                    r = slice(c * CH, (c + 1) * CH)
                    x1 = x1_src[r, lanes(t)]
                    h2 = _rb(_rb(_rb(_rb(x1 - mb[t]) * invs[t]) * col_buf[2, r, :]) + col_buf[1, r, :])
                    tr = h2 * col_buf[4, r, :]
                    acc[t] = tr if acc[t] is None else acc[t] + tr
                    hb = h2 + h2 * 0.0
                    outs.append(x1 + _rb(col_buf[3, r, :] * hb))
                    h_dst[r, lanes(t)] = (lax.bitcast_convert_type(h2, jnp.int32)
                                          | lax.shift_right_logical(lax.bitcast_convert_type(x1, jnp.int32), 16))
                out_buf[p * NLB + t, 16 * c2:16 * c2 + 16, :] = jnp.concatenate(outs, axis=0).astype(BF16)
        return [_sort_key(_rb(jnp.sum(acc[t], axis=0, keepdims=True)), (p * NLB + t) * TB + lane_id)
                for t in range(NLB)]

    def stage_d(p, t, h_src):
        xh_buf[pl.ds(pl.multiple_of((p * NLB + t) * TB, TB), TB), :] = h_src[:, lanes(t)].T

    def merge_top(keys):
        cands = [top_buf[...]] + list(keys)
        top = jnp.zeros((1, TB), F32)
        for t in range(TOPK):
            m = jnp.max(functools.reduce(jnp.maximum, cands), axis=1, keepdims=True)
            top = jnp.where(lane_id == t, m, top)
            cands = [jnp.where(c_ == m, 0.0, c_) for c_ in cands]
        top_buf[...] = top

    WD_PER_BLOCK = -(-(F // 128) // (NOB - 1))

    def wd_transpose(i):
        cols = pl.ds(pl.multiple_of(i * 128, 128), 128)
        wdn_buf[cols, :] = wd_buf[:, cols].T

    def op_block(b, carry):
        p = b - 1
        z = b & 1
        bA, bB, bH = acc_buf.at[z], x1t_buf.at[z], h2t_buf.at[z]
        bX, bXn = att_buf.at[z], att_buf.at[1 - z]
        RA, RB = 2, 3
        cur = bA
        accumulate(bA, None, part_of(b, 0))
        means = stage_a(p, bX, bB)
        for g in range(1, NG - 1):
            if g == RA:
                accumulate(bX, cur, part_of(b, g))
                cur = bX
                invs = stage_b(bB, means)
            elif g == RB:
                keys = stage_c(p, bB, means, invs, bH)
                accumulate(bB, cur, part_of(b, g))
                cur = bB
            else:
                accumulate(cur, cur, part_of(b, g))
        for t in range(NLB):
            stage_d(p, t, bH)
        for u in range(WD_PER_BLOCK):
            wd_transpose(jnp.minimum(p * WD_PER_BLOCK + u, F // 128 - 1))
        merge_top(keys)
        accumulate(bXn, cur, part_of(b, NG - 1))
        for t in range(NLB):
            d_out(p * NLB + t).start()
        return carry

    top_buf[...] = jnp.zeros((1, TB), F32)
    accumulate(acc_buf.at[0], None, part_of(0, 0))
    for g in range(1, NG - 1):
        accumulate(acc_buf.at[0], acc_buf.at[0], part_of(0, g))
    accumulate(att_buf.at[1], acc_buf.at[0], part_of(0, NG - 1))
    lax.fori_loop(1, NOB, op_block, 0)
    zl = NOB & 1
    means = stage_a(NOB - 1, att_buf.at[zl], x1t_buf.at[zl])
    invs = stage_b(x1t_buf.at[zl], means)
    last_keys = stage_c(NOB - 1, x1t_buf.at[zl], means, invs, h2t_buf.at[zl])
    for t in range(NLB):
        d_out((NOB - 1) * NLB + t).start()

    top_bits = lax.bitcast_convert_type(top_buf[...], jnp.int32)
    for t in range(TOPK):
        top_smem[t] = top_bits[0, t]
    for t in range(NLB):
        key_buf[t:t + 1, :] = last_keys[t]

    def pull_cond(state):
        n, go = state
        return go

    def pull_body(state):
        n, _ = state
        kv = key_buf[...]
        m = jnp.max(jnp.max(kv, axis=0, keepdims=True), axis=1, keepdims=True)
        m_bits = lax.bitcast_convert_type(m, jnp.int32)[0, 0]
        slot = TOPK - 1 - n
        better = m_bits > top_smem[slot]

        @pl.when(better)
        def _():
            top_smem[slot] = m_bits
            key_buf[...] = jnp.where(kv == m, 0.0, kv)

        n1 = n + better.astype(jnp.int32)
        return n1, jnp.logical_and(better, n1 < TOPK)

    n_new, _ = lax.while_loop(pull_cond, pull_body, (jnp.int32(0), jnp.bool_(True)))
    @pl.when(n_new > 0)
    def _():
        for t in range(NLB):
            stage_d(NOB - 1, t, h2t_buf.at[zl])

    row8 = lax.broadcasted_iota(jnp.int32, (TOPK, 128), 0)
    kb = jnp.zeros((TOPK, 128), jnp.int32)
    for t in range(TOPK):
        kt = top_smem[t] - KEY_BIAS
        idx_smem[t] = jnp.clip((S - 1) - (kt & (S - 1)), 0, S - 1)
        kb = jnp.where(row8 == t, kt, kb)
    srt = lax.shift_right_logical(kb, 11)
    u16 = jnp.where(srt >= 0x8000, srt & 0x7FFF, 0xFFFF - srt)
    r_sel = lax.bitcast_convert_type(lax.shift_left(u16, 16), F32)[:, 0:1]

    for t in range(TOPK):
        xs_buf[pl.ds(t, 1), :] = xh_buf[pl.ds(idx_smem[t], 1), :]
    xw = xs_buf[...]
    xs = lax.bitcast_convert_type(xw & jnp.int32(-65536), F32)
    x1s = lax.bitcast_convert_type(lax.shift_left(xw, 16), F32)
    xs_b = xs.astype(BF16)

    d_wg.wait()
    d_wu.wait()
    g = _rb(_dot(xs_b, wg_buf[...]))
    u = _rb(_dot(xs_b, wu_buf[...]))
    act = _rb(_rb(g * _sigmoid_b(g)) * u).astype(BF16)
    y = _rb(_dot(act, wdn_buf[...]))
    y = _rb(y * _sigmoid_b(r_sel))
    hb_sel = _rb(xs + _rb(_rb(xs * 0.0) + y))
    new = x1s + _rb(gb_buf[...] * hb_sel)
    new_t = jnp.concatenate([new, jnp.zeros((128 - TOPK, D), F32)], axis=0).T
    new_w = pltpu.bitcast(new_t.astype(BF16), jnp.int32)

    lane = lax.broadcasted_iota(jnp.int32, (D // 2, 128), 1)
    blk = [idx_smem[t] // TB for t in range(TOPK)]
    for b in range(NTB):
        d_out(b).wait()
    for t in range(TOPK):
        ln_t = idx_smem[t] % TB
        rolled = pltpu.roll(new_w, (ln_t + (TB - t)) % TB, axis=1)
        out32[blk[t]] = jnp.where(lane == ln_t, rolled, out32[blk[t]])

    def d_patch(t):
        return cp(out_buf.at[blk[t]], out_hbm.at[:, pl.ds(pl.multiple_of(blk[t] * TB, TB), TB)], sem_patch.at[t])

    first = []
    for t in range(TOPK):
        f = blk[t] >= 0
        for t2 in range(t):
            f = jnp.logical_and(f, blk[t] != blk[t2])
        first.append(f)
    for t in range(TOPK):
        pl.when(first[t])(lambda t=t: d_patch(t).start())
    for t in range(TOPK):
        pl.when(first[t])(lambda t=t: d_patch(t).wait())


@jax.jit
def pallas_adaLN_cond__gqa_block_cached__moe_arch_mod__prompt_kernel(
    A_x, A_k_cache, A_v_cache, A_wq, A_wo, B_x, B_w_r, B_w_gate, B_w_up, B_w_down, c, w_mod,
):
    del B_x
    xt = A_x.reshape(S, D).T
    k = A_k_cache.reshape(HKV, S, DH)
    v = A_v_cache.reshape(HKV, S, DH)
    hbm = pl.BlockSpec(memory_space=pl.ANY)
    out = pl.pallas_call(
        _kernel,
        in_specs=[hbm] * 11,
        out_specs=hbm,
        out_shape=jax.ShapeDtypeStruct((D, S), BF16),
        scratch_shapes=[
            pltpu.VMEM((NTB, D, TB), BF16),
            pltpu.VMEM((NP, S, 128), BF16),
            pltpu.VMEM((S // 2, 128), BF16),
            pltpu.VMEM((2 * S, DH), BF16),
            pltpu.VMEM((HKV, S, DH), BF16),
            pltpu.VMEM((HKV, S, DH), BF16),
            pltpu.VMEM((HKV, D, 2 * DH), BF16),
            pltpu.VMEM((HQ, D, DH), BF16),
            pltpu.VMEM((D,), BF16),
            pltpu.VMEM((D, F), BF16),
            pltpu.VMEM((D, F), BF16),
            pltpu.VMEM((D, F), BF16),
            pltpu.VMEM((F, D), BF16),
            pltpu.VMEM((1, D), BF16),
            pltpu.VMEM((D, 2 * D), BF16),
            pltpu.VMEM((D, 4 * D), BF16),
            pltpu.VMEM((HKV, 2 * S, DH), BF16),
            pltpu.VMEM((S, D), jnp.int32),
            pltpu.VMEM((NTB, D, TB), BF16),
            pltpu.VMEM((OB // TB, TB), F32),
            pltpu.VMEM((1, TB), F32),
            pltpu.VMEM((2, D, OB), F32),
            pltpu.VMEM((2, D, OB), F32),
            pltpu.VMEM((2, D, OB), F32),
            pltpu.VMEM((2, D, OB), jnp.int32),
            pltpu.VMEM((5, D, TB), F32),
            pltpu.VMEM((1, D), F32),
            pltpu.VMEM((TOPK, D), jnp.int32),
            pltpu.SMEM((TOPK,), jnp.int32),
            pltpu.SMEM((TOPK,), jnp.int32),
            pltpu.SemaphoreType.DMA((9,)),
            pltpu.SemaphoreType.DMA((HKV,)),
            pltpu.SemaphoreType.DMA((HKV,)),
            pltpu.SemaphoreType.DMA((HKV,)),
            pltpu.SemaphoreType.DMA((NTB,)),
            pltpu.SemaphoreType.DMA((NTB,)),
            pltpu.SemaphoreType.DMA((TOPK,)),
        ],
        compiler_params=pltpu.CompilerParams(vmem_limit_bytes=120 * 1024 * 1024, disable_bounds_checks=True,
                                             disable_semaphore_checks=True),
    )(xt, k, v, A_wq, A_wo.T, B_w_r, B_w_gate, B_w_up, B_w_down.T, c, w_mod)
    return out.T.reshape(1, S, D)
```

```python
import functools
import math

import jax
import jax.numpy as jnp
import numpy as np
from jax import lax
from jax.experimental import pallas as pl
from jax.experimental.pallas import tpu as pltpu

S = 2048
D = 576
HQ = 32
HKV = 16
DH = 128
F = 4608
TOPK = 8
EPS = 1e-5
TB = 128
NTB = S // TB
OB = 256
NP = D // 128
DM = NP * 128

RBLK = [288] + [272] * 14

F32 = jnp.float32
BF16 = jnp.bfloat16
NT_DIMS = (((1,), (1,)), ((), ()))
NN_DIMS = (((1,), (0,)), ((), ()))


def _rb(v):
    return v.astype(BF16).astype(F32)


def _dot(a, b, dims=NN_DIMS):
    return lax.dot_general(a, b, dims, preferred_element_type=F32)


def _sigmoid_b(g):
    return _rb(1.0 / _rb(1.0 + _rb(jnp.exp(-g))))


def _ln1_t(xf):
    inv_d = np.float32(1.0 / D)
    m32 = jnp.sum(xf, axis=0, keepdims=True) * inv_d
    cen = xf - m32
    v = jnp.sum(cen * cen, axis=0, keepdims=True) * inv_d
    return cen * lax.rsqrt(v + np.float32(EPS))


def _col(row):
    return jnp.broadcast_to(row, (128, D)).T


KEY_BIAS = 0x20000000


def _sort_key(r, tok):
    bits = lax.bitcast_convert_type(r, jnp.int32)
    u = lax.shift_right_logical(bits, 16)
    u = jnp.where(u == 0x8000, 0, u)
    srt = jnp.where(u >= 0x8000, 0xFFFF - u, u | 0x8000)
    srt = jnp.where(r != r, 0, srt)
    key = lax.shift_left(srt, 11) | (S - 1 - tok)
    return lax.bitcast_convert_type(key + KEY_BIAS, F32)


def _kernel(xt_hbm, k_hbm, v_hbm, wq_hbm, wot_hbm, wr_hbm, wg_hbm, wu_hbm, wdt_hbm, c_hbm, wmod_hbm,
            out_hbm,
            x_buf, h_buf, ht_buf, q_buf, k_buf, v_buf, wq_buf, wo_buf, wr_buf, wg_buf, wu_buf, wd_buf, wdn_buf, c_buf,
            wma_buf, wmb_buf, o2_buf, xh_buf, out_buf, key_buf, top_buf, att_buf, acc_buf, x1t_buf, h2t_buf, col_buf, gb_buf, xs_buf, top_smem,
            sem_misc, sem_k, sem_v, sem_q, sem_x, sem_out, sem_patch):
    k32 = k_buf.bitcast(jnp.int32)
    v32 = v_buf.bitcast(jnp.int32)
    o32 = o2_buf.bitcast(jnp.int32)
    h32 = h_buf.bitcast(jnp.int32)
    ht32 = ht_buf.bitcast(jnp.int32)
    q32 = q_buf.bitcast(jnp.int32)
    wo32 = wo_buf.bitcast(jnp.int32)
    out32 = out_buf.bitcast(jnp.int32)

    def as_bf16(v):
        return pltpu.bitcast(v, BF16)

    def cp(src, dst, sem):
        return pltpu.make_async_copy(src, dst, sem)

    d_c = cp(c_hbm, c_buf, sem_misc.at[0])
    d_wma = cp(wmod_hbm.at[:, pl.ds(0, 2 * D)], wma_buf, sem_misc.at[1])
    d_wmb = cp(wmod_hbm.at[:, pl.ds(2 * D, 4 * D)], wmb_buf, sem_misc.at[3])

    class _Group:
        def __init__(self, copies):
            self.copies = copies

        def start(self):
            for c in self.copies:
                c.start()

        def wait(self):
            for c in self.copies:
                c.wait()

    d_wo = _Group([cp(wot_hbm.at[:, pl.ds(h * DH, DH)], wo_buf.at[h], sem_misc.at[4]) for h in range(HQ)])
    d_wr = cp(wr_hbm, wr_buf, sem_misc.at[5])
    d_wg = cp(wg_hbm, wg_buf, sem_misc.at[6])
    d_wu = cp(wu_hbm, wu_buf, sem_misc.at[7])
    d_wd = cp(wdt_hbm, wd_buf, sem_misc.at[8])

    def d_x(b):
        return cp(xt_hbm.at[:, pl.ds(pl.multiple_of(b * TB, TB), TB)], x_buf.at[b], sem_x.at[b])

    def d_out(b):
        return cp(out_buf.at[b], out_hbm.at[:, pl.ds(pl.multiple_of(b * TB, TB), TB)], sem_out.at[b])

    def d_k(j):
        return cp(k_hbm.at[j], k_buf.at[j], sem_k.at[j])

    def d_v(j):
        return cp(v_hbm.at[j], v_buf.at[j], sem_v.at[j])

    def d_q(j):
        return cp(wq_hbm.at[:, pl.ds(pl.multiple_of(j * 2 * DH, 2 * DH), 2 * DH)], wq_buf.at[j], sem_q.at[j])

    LNG = 4
    d_c.start()
    d_wma.start()
    for b in range(NTB):
        d_x(b).start(priority=1)
    d_q(0).start(priority=1)
    d_k(0).start(priority=1)
    d_v(0).start(priority=1)

    d_c.wait()
    cf = c_buf[...].astype(F32)
    sc = _rb(cf * _sigmoid_b(cf))
    sc8 = jnp.broadcast_to(sc, (8, D)).astype(BF16)
    d_wma.wait()
    mod_a = _rb(_dot(sc8, wma_buf[...]))
    col_buf[0] = _col(_rb(1.0 + mod_a[0:1, D:2 * D]))
    col_buf[1] = _col(mod_a[0:1, 0:D])

    def ln1_body(g, carry):
        for t in range(LNG):
            d_x(g * LNG + t).wait()
        tails = []
        for t in range(LNG):
            b = g * LNG + t
            xf = x_buf[b].astype(F32)
            ht = _ln1_t(xf) * col_buf[0] + col_buf[1]
            hv = ht[:DM, :].T.astype(BF16)
            rows = pl.ds(pl.multiple_of(b * TB, TB), TB)
            for p in range(NP):
                h_buf[p, rows, :] = hv[:, p * 128:(p + 1) * 128]
            tails.append(ht[DM:, :])
        for t in range(2):
            rows = pl.ds(pl.multiple_of((2 * g + t) * TB, TB), TB)
            ht_buf[rows, :] = jnp.concatenate([tails[t], tails[t + 2]], axis=0).T.astype(BF16)
        return carry

    lax.fori_loop(0, NTB // LNG, ln1_body, 0)

    q_scale = np.float32(DH ** -0.5 * math.log2(math.e))

    def prefetch(j):
        d_q(j).start(priority=1)
        d_k(j).start(priority=1)
        d_v(j).start(priority=1)

    def att_body(j, carry):
        d_q(j).wait()
        pl.when(j > 0)(lambda: d_k(j).wait())
        pl.when(j > 0)(lambda: d_v(j).wait())

        wqv = wq_buf[j]
        w_tail = wqv[DM:, :]
        zero = jnp.zeros_like(w_tail)
        w2 = jnp.concatenate([jnp.concatenate([w_tail, zero], axis=1),
                              jnp.concatenate([zero, w_tail], axis=1)], axis=0)
        RQ = 256
        for g in range(S // (2 * RQ)):
            ht = as_bf16(ht32[pl.ds(g * (RQ // 2), RQ // 2), :])
            q_tail = _dot(ht, w2)
            for u in range(2):
                b = 2 * g + u
                rows = pl.ds(b * RQ, RQ)
                rows2 = pl.ds(b * (RQ // 2), RQ // 2)
                hm = jnp.concatenate([as_bf16(h32[p, rows2, :]) for p in range(NP)], axis=1)
                qf = _dot(hm, wqv[:DM, :]) + q_tail[:, u * 2 * DH:(u + 1) * 2 * DH]
                q2 = (qf * q_scale).astype(BF16)
                q_buf[pl.ds(b * RQ, RQ), :] = q2[:, :DH]
                q_buf[pl.ds(S + b * RQ, RQ), :] = q2[:, DH:]
        r0 = 0
        for rsz in RBLK:
            rows = pl.ds(r0, rsz)
            q = as_bf16(q32[pl.ds(r0 // 2, rsz // 2), :])
            s = _dot(q, as_bf16(k32[j]), NT_DIMS)
            m = jnp.max(s, axis=-1, keepdims=True)
            p = jnp.exp2(s - m)
            l = jnp.sum(p, axis=-1, keepdims=True)
            o = _dot(p.astype(BF16), as_bf16(v32[j]))
            o2_buf[j, rows, :] = (o * pltpu.reciprocal(l, approx=True)).astype(BF16)
            r0 += rsz

        pl.when(j + 2 < HKV)(lambda: prefetch(j + 2))
        pl.when(j == 1)(d_wmb.start)
        pl.when(j == 1)(d_wr.start)
        pl.when(j == 3)(d_wo.start)
        pl.when(j == 5)(d_wg.start)
        pl.when(j == 7)(d_wu.start)
        pl.when(j == 9)(d_wd.start)
        return carry

    d_k(0).wait()
    d_v(0).wait()
    prefetch(1)
    lax.fori_loop(0, HKV, att_body, 0)

    d_wmb.wait()
    d_wr.wait()
    d_wo.wait()
    d_wd.wait()
    mod_b = _rb(_dot(sc8, wmb_buf[...]))
    gb = mod_b[0:1, 3 * D:4 * D]
    gb_buf[...] = gb
    col_buf[0] = _col(mod_b[0:1, 0:D])
    col_buf[1] = _col(mod_b[0:1, D:2 * D])
    col_buf[2] = _col(_rb(1.0 + mod_b[0:1, 2 * D:3 * D]))
    col_buf[3] = _col(gb)
    col_buf[4] = _col(wr_buf[...].astype(F32).reshape(1, D))

    lane_id = lax.broadcasted_iota(jnp.int32, (1, TB), 1)

    NG = 8
    HG = HQ // NG
    CH = 8
    NC = D // CH
    NLB = OB // TB
    NOB = S // OB
    inv_d = np.float32(1.0 / D)
    eps_b = np.float32(np.float32(EPS).astype(jnp.bfloat16))

    def lanes(t):
        return slice(t * TB, (t + 1) * TB)

    def part_of(b, g):
        def tok2_of(h):
            return pl.ds(pl.multiple_of((h % 2) * (S // 2) + b * (OB // 2), OB // 2), OB // 2)
        heads = range(g * HG, (g + 1) * HG)
        o_cat = jnp.concatenate([as_bf16(o32[h // 2, tok2_of(h), :]) for h in heads], axis=1)
        wo_t = jnp.concatenate([as_bf16(wo32[h]) for h in heads], axis=1)
        return _dot(wo_t, o_cat, NT_DIMS)

    def accumulate(dst, src, part):
        for c in range(NC):
            r = slice(c * CH, (c + 1) * CH)
            dst[r, :] = part[r, :] if src is None else src[r, :] + part[r, :]

    def stage_a(p, att, x1_dst):
        means = []
        for t in range(NLB):
            acc = None
            for c in range(NC):
                r = slice(c * CH, (c + 1) * CH)
                c16 = slice((c // 2) * 16, (c // 2) * 16 + 16)
                xv = x_buf[p * NLB + t, c16, :].astype(F32)[(c % 2) * 8:(c % 2) * 8 + 8, :]
                x1 = _rb(xv + col_buf[0, r, :] * att[r, lanes(t)])
                x1_dst[r, lanes(t)] = x1
                acc = x1 if acc is None else acc + x1
            means.append(jnp.sum(acc, axis=0, keepdims=True) * inv_d)
        return means

    def stage_b(x1_src, means):
        invs = []
        for t in range(NLB):
            acc = None
            for c in range(NC):
                r = slice(c * CH, (c + 1) * CH)
                cen = x1_src[r, lanes(t)] - means[t]
                acc = cen * cen if acc is None else acc + cen * cen
            v = _rb(jnp.sum(acc, axis=0, keepdims=True) * inv_d)
            invs.append(1.0 / _rb(jnp.sqrt(_rb(v + eps_b))))
        return invs

    def stage_c(p, x1_src, means, invs, h_dst):
        mb = [_rb(m) for m in means]
        acc = [None] * NLB
        for c2 in range(NC // 2):
            for t in range(NLB):
                outs = []
                for c in (2 * c2, 2 * c2 + 1):
                    r = slice(c * CH, (c + 1) * CH)
                    x1 = x1_src[r, lanes(t)]
                    h2 = _rb(_rb(_rb(_rb(x1 - mb[t]) * invs[t]) * col_buf[2, r, :]) + col_buf[1, r, :])
                    tr = h2 * col_buf[4, r, :]
                    acc[t] = tr if acc[t] is None else acc[t] + tr
                    hb = h2 + h2 * 0.0
                    outs.append(x1 + _rb(col_buf[3, r, :] * hb))
                    h_dst[r, lanes(t)] = (lax.bitcast_convert_type(h2, jnp.int32)
                                          | lax.shift_right_logical(lax.bitcast_convert_type(x1, jnp.int32), 16))
                out_buf[p * NLB + t, 16 * c2:16 * c2 + 16, :] = jnp.concatenate(outs, axis=0).astype(BF16)
        return [_sort_key(_rb(jnp.sum(acc[t], axis=0, keepdims=True)), (p * NLB + t) * TB + lane_id)
                for t in range(NLB)]

    def stage_d(p, t, h_src):
        xh_buf[pl.ds(pl.multiple_of((p * NLB + t) * TB, TB), TB), :] = h_src[:, lanes(t)].T

    def merge_top(keys):
        cands = [top_buf[...]] + list(keys)
        top = jnp.zeros((1, TB), F32)
        for t in range(TOPK):
            m = jnp.max(functools.reduce(jnp.maximum, cands), axis=1, keepdims=True)
            top = jnp.where(lane_id == t, m, top)
            cands = [jnp.where(c_ == m, 0.0, c_) for c_ in cands]
        top_buf[...] = top

    WD_PER_BLOCK = -(-(F // 128) // (NOB - 1))

    def wd_transpose(i):
        cols = pl.ds(pl.multiple_of(i * 128, 128), 128)
        wdn_buf[cols, :] = wd_buf[:, cols].T

    def op_block(b, carry):
        p = b - 1
        z = b & 1
        bA, bB, bH = acc_buf.at[z], x1t_buf.at[z], h2t_buf.at[z]
        bX, bXn = att_buf.at[z], att_buf.at[1 - z]
        RA, RB = 2, 3
        cur = bA
        accumulate(bA, None, part_of(b, 0))
        means = stage_a(p, bX, bB)
        for g in range(1, NG - 1):
            if g == RA:
                accumulate(bX, cur, part_of(b, g))
                cur = bX
                invs = stage_b(bB, means)
            elif g == RB:
                keys = stage_c(p, bB, means, invs, bH)
                accumulate(bB, cur, part_of(b, g))
                cur = bB
            else:
                accumulate(cur, cur, part_of(b, g))
        for t in range(NLB):
            stage_d(p, t, bH)
        for u in range(WD_PER_BLOCK):
            wd_transpose(jnp.minimum(p * WD_PER_BLOCK + u, F // 128 - 1))
        merge_top(keys)
        accumulate(bXn, cur, part_of(b, NG - 1))
        for t in range(NLB):
            d_out(p * NLB + t).start()
        return carry

    top_buf[...] = jnp.zeros((1, TB), F32)
    accumulate(acc_buf.at[0], None, part_of(0, 0))
    for g in range(1, NG - 1):
        accumulate(acc_buf.at[0], acc_buf.at[0], part_of(0, g))
    accumulate(att_buf.at[1], acc_buf.at[0], part_of(0, NG - 1))
    lax.fori_loop(1, NOB, op_block, 0)
    zl = NOB & 1
    means = stage_a(NOB - 1, att_buf.at[zl], x1t_buf.at[zl])
    invs = stage_b(x1t_buf.at[zl], means)
    last_keys = stage_c(NOB - 1, x1t_buf.at[zl], means, invs, h2t_buf.at[zl])
    for t in range(NLB):
        d_out((NOB - 1) * NLB + t).start()

    top_bits = lax.bitcast_convert_type(top_buf[...], jnp.int32)
    for t in range(TOPK):
        top_smem[t] = top_bits[0, t]
    for t in range(NLB):
        key_buf[t:t + 1, :] = last_keys[t]

    def pull_cond(state):
        n, go = state
        return go

    def pull_body(state):
        n, _ = state
        kv = key_buf[...]
        m = jnp.max(jnp.max(kv, axis=0, keepdims=True), axis=1, keepdims=True)
        m_bits = lax.bitcast_convert_type(m, jnp.int32)[0, 0]
        slot = TOPK - 1 - n
        better = m_bits > top_smem[slot]

        @pl.when(better)
        def _():
            top_smem[slot] = m_bits
            key_buf[...] = jnp.where(kv == m, 0.0, kv)

        n1 = n + better.astype(jnp.int32)
        return n1, jnp.logical_and(better, n1 < TOPK)

    lax.while_loop(pull_cond, pull_body, (jnp.int32(0), jnp.bool_(True)))

    row8 = lax.broadcasted_iota(jnp.int32, (TOPK, 128), 0)
    kb = jnp.zeros((TOPK, 128), jnp.int32)
    idx = []
    for t in range(TOPK):
        kt = top_smem[t] - KEY_BIAS
        idx.append(jnp.clip((S - 1) - (kt & (S - 1)), 0, S - 1))
        kb = jnp.where(row8 == t, kt, kb)
    blk = [i // TB for i in idx]

    for t in range(NLB):
        hit = functools.reduce(jnp.logical_or, [b_ == (NOB - 1) * NLB + t for b_ in blk])
        pl.when(hit)(lambda t=t: stage_d(NOB - 1, t, h2t_buf.at[zl]))
    srt = lax.shift_right_logical(kb, 11)
    u16 = jnp.where(srt >= 0x8000, srt & 0x7FFF, 0xFFFF - srt)
    r_sel = lax.bitcast_convert_type(lax.shift_left(u16, 16), F32)[:, 0:1]

    for t in range(TOPK):
        xs_buf[pl.ds(t, 1), :] = xh_buf[pl.ds(idx[t], 1), :]
    xw = xs_buf[...]
    xs = lax.bitcast_convert_type(xw & jnp.int32(-65536), F32)
    x1s = lax.bitcast_convert_type(lax.shift_left(xw, 16), F32)
    xs_b = xs.astype(BF16)

    d_wg.wait()
    d_wu.wait()
    g = _rb(_dot(xs_b, wg_buf[...]))
    u = _rb(_dot(xs_b, wu_buf[...]))
    act = _rb(_rb(g * _sigmoid_b(g)) * u).astype(BF16)
    y = _rb(_dot(act, wdn_buf[...]))
    y = _rb(y * _sigmoid_b(r_sel))
    hb_sel = _rb(xs + _rb(_rb(xs * 0.0) + y))
    new = x1s + _rb(gb_buf[...] * hb_sel)
    new_t = jnp.concatenate([new, jnp.zeros((128 - TOPK, D), F32)], axis=0).T
    new_w = pltpu.bitcast(new_t.astype(BF16), jnp.int32)

    lane = lax.broadcasted_iota(jnp.int32, (D // 2, 128), 1)
    for b in range(NTB):
        d_out(b).wait()

    def d_patch(t):
        return cp(out_buf.at[blk[t]], out_hbm.at[:, pl.ds(pl.multiple_of(blk[t] * TB, TB), TB)], sem_patch.at[t])

    last = []
    for t in range(TOPK):
        f = blk[t] >= 0
        for t2 in range(t + 1, TOPK):
            f = jnp.logical_and(f, blk[t] != blk[t2])
        last.append(f)
    for t in range(TOPK):
        ln_t = idx[t] % TB
        rolled = pltpu.roll(new_w, (ln_t + (TB - t)) % TB, axis=1)
        out32[blk[t]] = jnp.where(lane == ln_t, rolled, out32[blk[t]])
        pl.when(last[t])(lambda t=t: d_patch(t).start())
    for t in range(TOPK):
        pl.when(last[t])(lambda t=t: d_patch(t).wait())


@jax.jit
def pallas_adaLN_cond__gqa_block_cached__moe_arch_mod__prompt_kernel(
    A_x, A_k_cache, A_v_cache, A_wq, A_wo, B_x, B_w_r, B_w_gate, B_w_up, B_w_down, c, w_mod,
):
    del B_x
    xt = A_x.reshape(S, D).T
    k = A_k_cache.reshape(HKV, S, DH)
    v = A_v_cache.reshape(HKV, S, DH)
    hbm = pl.BlockSpec(memory_space=pl.ANY)
    out = pl.pallas_call(
        _kernel,
        in_specs=[hbm] * 11,
        out_specs=hbm,
        out_shape=jax.ShapeDtypeStruct((D, S), BF16),
        scratch_shapes=[
            pltpu.VMEM((NTB, D, TB), BF16),
            pltpu.VMEM((NP, S, 128), BF16),
            pltpu.VMEM((S // 2, 128), BF16),
            pltpu.VMEM((2 * S, DH), BF16),
            pltpu.VMEM((HKV, S, DH), BF16),
            pltpu.VMEM((HKV, S, DH), BF16),
            pltpu.VMEM((HKV, D, 2 * DH), BF16),
            pltpu.VMEM((HQ, D, DH), BF16),
            pltpu.VMEM((D,), BF16),
            pltpu.VMEM((D, F), BF16),
            pltpu.VMEM((D, F), BF16),
            pltpu.VMEM((D, F), BF16),
            pltpu.VMEM((F, D), BF16),
            pltpu.VMEM((1, D), BF16),
            pltpu.VMEM((D, 2 * D), BF16),
            pltpu.VMEM((D, 4 * D), BF16),
            pltpu.VMEM((HKV, 2 * S, DH), BF16),
            pltpu.VMEM((S, D), jnp.int32),
            pltpu.VMEM((NTB, D, TB), BF16),
            pltpu.VMEM((OB // TB, TB), F32),
            pltpu.VMEM((1, TB), F32),
            pltpu.VMEM((2, D, OB), F32),
            pltpu.VMEM((2, D, OB), F32),
            pltpu.VMEM((2, D, OB), F32),
            pltpu.VMEM((2, D, OB), jnp.int32),
            pltpu.VMEM((5, D, TB), F32),
            pltpu.VMEM((1, D), F32),
            pltpu.VMEM((TOPK, D), jnp.int32),
            pltpu.SMEM((TOPK,), jnp.int32),
            pltpu.SemaphoreType.DMA((9,)),
            pltpu.SemaphoreType.DMA((HKV,)),
            pltpu.SemaphoreType.DMA((HKV,)),
            pltpu.SemaphoreType.DMA((HKV,)),
            pltpu.SemaphoreType.DMA((NTB,)),
            pltpu.SemaphoreType.DMA((NTB,)),
            pltpu.SemaphoreType.DMA((TOPK,)),
        ],
        compiler_params=pltpu.CompilerParams(vmem_limit_bytes=120 * 1024 * 1024, disable_bounds_checks=True,
                                             disable_semaphore_checks=True),
    )(xt, k, v, A_wq, A_wo.T, B_w_r, B_w_gate, B_w_up, B_w_down.T, c, w_mod)
    return out.T.reshape(1, S, D)
```

```python
import functools
import math

import jax
import jax.numpy as jnp
import numpy as np
from jax import lax
from jax.experimental import pallas as pl
from jax.experimental.pallas import tpu as pltpu

S = 2048
D = 576
HQ = 32
HKV = 16
DH = 128
F = 4608
TOPK = 8
EPS = 1e-5
TB = 128
NTB = S // TB
OB = 256
NP = D // 128
DM = NP * 128
RQ = 256
LNG = 4
RBLK = [272, 288, 288] + [272] * 11 + [256]
assert sum(RBLK) == 2 * S and LNG * TB == 2 * RQ

F32 = jnp.float32
BF16 = jnp.bfloat16
NT_DIMS = (((1,), (1,)), ((), ()))
NN_DIMS = (((1,), (0,)), ((), ()))


def _rb(v):
    return v.astype(BF16).astype(F32)


def _dot(a, b, dims=NN_DIMS):
    return lax.dot_general(a, b, dims, preferred_element_type=F32)


def _sigmoid_b(g):
    return _rb(1.0 / _rb(1.0 + _rb(jnp.exp(-g))))


def _ln1_t(xf):
    inv_d = np.float32(1.0 / D)
    m32 = jnp.sum(xf, axis=0, keepdims=True) * inv_d
    cen = xf - m32
    v = jnp.sum(cen * cen, axis=0, keepdims=True) * inv_d
    return cen * lax.rsqrt(v + np.float32(EPS))


def _col(row):
    return jnp.broadcast_to(row, (128, D)).T


KEY_BIAS = 0x20000000


def _sort_key(r, tok):
    bits = lax.bitcast_convert_type(r, jnp.int32)
    u = lax.shift_right_logical(bits, 16)
    u = jnp.where(u == 0x8000, 0, u)
    srt = jnp.where(u >= 0x8000, 0xFFFF - u, u | 0x8000)
    srt = jnp.where(r != r, 0, srt)
    key = lax.shift_left(srt, 11) | (S - 1 - tok)
    return lax.bitcast_convert_type(key + KEY_BIAS, F32)


def _kernel(xt_hbm, k_hbm, v_hbm, wq_hbm, wot_hbm, wr_hbm, wg_hbm, wu_hbm, wdt_hbm, c_hbm, wmod_hbm,
            out_hbm,
            x_buf, h_buf, ht_buf, q_buf, k_buf, v_buf, wq_buf, wo_buf, wr_buf, wg_buf, wu_buf, wd_buf, wdn_buf, c_buf,
            wma_buf, wmb_buf, o2_buf, xh_buf, out_buf, key_buf, top_buf, att_buf, acc_buf, x1t_buf, h2t_buf, col_buf, gb_buf, xs_buf, top_smem,
            sem_misc, sem_k, sem_v, sem_q, sem_x, sem_out, sem_patch):
    k32 = k_buf.bitcast(jnp.int32)
    v32 = v_buf.bitcast(jnp.int32)
    o32 = o2_buf.bitcast(jnp.int32)
    h32 = h_buf.bitcast(jnp.int32)
    ht32 = ht_buf.bitcast(jnp.int32)
    q32 = q_buf.bitcast(jnp.int32)
    wo32 = wo_buf.bitcast(jnp.int32)
    out32 = out_buf.bitcast(jnp.int32)

    def as_bf16(v):
        return pltpu.bitcast(v, BF16)

    def cp(src, dst, sem):
        return pltpu.make_async_copy(src, dst, sem)

    d_c = cp(c_hbm, c_buf, sem_misc.at[0])
    d_wma = cp(wmod_hbm.at[:, pl.ds(0, 2 * D)], wma_buf, sem_misc.at[1])
    d_wmb = cp(wmod_hbm.at[:, pl.ds(2 * D, 4 * D)], wmb_buf, sem_misc.at[2])

    class _Group:
        def __init__(self, copies):
            self.copies = copies

        def start(self):
            for c in self.copies:
                c.start()

        def wait(self):
            for c in self.copies:
                c.wait()

    d_wo = _Group([cp(wot_hbm.at[:, pl.ds(h * DH, DH)], wo_buf.at[h], sem_misc.at[3]) for h in range(HQ)])
    d_wr = cp(wr_hbm, wr_buf, sem_misc.at[4])
    d_wg = cp(wg_hbm, wg_buf, sem_misc.at[5])
    d_wu = cp(wu_hbm, wu_buf, sem_misc.at[6])
    d_wd = cp(wdt_hbm, wd_buf, sem_misc.at[7])

    def d_x(b):
        return cp(xt_hbm.at[:, pl.ds(pl.multiple_of(b * TB, TB), TB)], x_buf.at[b], sem_x.at[b])

    def d_out(b):
        return cp(out_buf.at[b], out_hbm.at[:, pl.ds(pl.multiple_of(b * TB, TB), TB)], sem_out.at[b])

    def d_k(j):
        return cp(k_hbm.at[j], k_buf.at[j], sem_k.at[j])

    def d_v(j):
        return cp(v_hbm.at[j], v_buf.at[j], sem_v.at[j])

    def d_q(j):
        return cp(wq_hbm.at[:, pl.ds(pl.multiple_of(j * 2 * DH, 2 * DH), 2 * DH)], wq_buf.at[j], sem_q.at[j])

    d_c.start()
    d_wma.start()
    for b in range(NTB):
        d_x(b).start(priority=1)
    d_q(0).start(priority=1)
    d_k(0).start(priority=1)
    d_v(0).start(priority=1)

    d_c.wait()
    cf = c_buf[...].astype(F32)
    sc = _rb(cf * _sigmoid_b(cf))
    sc8 = jnp.broadcast_to(sc, (8, D)).astype(BF16)
    d_wma.wait()
    mod_a = _rb(_dot(sc8, wma_buf[...]))
    col_buf[0] = _col(_rb(1.0 + mod_a[0:1, D:2 * D]))
    col_buf[1] = _col(mod_a[0:1, 0:D])

    def ln1_body(g, carry):
        for t in range(LNG):
            d_x(g * LNG + t).wait()
        tails = []
        for t in range(LNG):
            b = g * LNG + t
            xf = x_buf[b].astype(F32)
            ht = _ln1_t(xf) * col_buf[0] + col_buf[1]
            hv = ht[:DM, :].T.astype(BF16)
            rows = pl.ds(pl.multiple_of(b * TB, TB), TB)
            for p in range(NP):
                h_buf[p, rows, :] = hv[:, p * 128:(p + 1) * 128]
            tails.append(ht[DM:, :])
        for t in range(2):
            rows = pl.ds(pl.multiple_of((2 * g + t) * TB, TB), TB)
            ht_buf[rows, :] = jnp.concatenate([tails[t], tails[t + 2]], axis=0).T.astype(BF16)
        return carry

    lax.fori_loop(0, NTB // LNG, ln1_body, 0)

    q_scale = np.float32(DH ** -0.5 * math.log2(math.e))

    def prefetch(j):
        d_q(j).start(priority=1)
        d_k(j).start(priority=1)
        d_v(j).start(priority=1)

    def att_body(j, carry):
        d_q(j).wait()
        pl.when(j > 0)(lambda: d_k(j).wait())
        pl.when(j > 0)(lambda: d_v(j).wait())

        wqv = wq_buf[j]
        w_tail = wqv[DM:, :]
        zero = jnp.zeros_like(w_tail)
        w2 = jnp.concatenate([jnp.concatenate([w_tail, zero], axis=1),
                              jnp.concatenate([zero, w_tail], axis=1)], axis=0)
        for g in range(S // (2 * RQ)):
            ht = as_bf16(ht32[pl.ds(g * (RQ // 2), RQ // 2), :])
            q_tail = _dot(ht, w2)
            for u in range(2):
                b = 2 * g + u
                rows = pl.ds(b * RQ, RQ)
                rows2 = pl.ds(b * (RQ // 2), RQ // 2)
                hm = jnp.concatenate([as_bf16(h32[p, rows2, :]) for p in range(NP)], axis=1)
                qf = _dot(hm, wqv[:DM, :]) + q_tail[:, u * 2 * DH:(u + 1) * 2 * DH]
                q2 = (qf * q_scale).astype(BF16)
                q_buf[pl.ds(b * RQ, RQ), :] = q2[:, :DH]
                q_buf[pl.ds(S + b * RQ, RQ), :] = q2[:, DH:]
        r0 = 0
        for rsz in RBLK:
            rows = pl.ds(r0, rsz)
            q = as_bf16(q32[pl.ds(r0 // 2, rsz // 2), :])
            s = _dot(q, as_bf16(k32[j]), NT_DIMS)
            m = jnp.max(s, axis=-1, keepdims=True)
            p = jnp.exp2(s - m)
            l = jnp.sum(p, axis=-1, keepdims=True)
            o = _dot(p.astype(BF16), as_bf16(v32[j]))
            o2_buf[j, rows, :] = (o * pltpu.reciprocal(l, approx=True)).astype(BF16)
            r0 += rsz

        pl.when(j + 2 < HKV)(lambda: prefetch(j + 2))
        pl.when(j == 1)(d_wmb.start)
        pl.when(j == 1)(d_wr.start)
        pl.when(j == 3)(d_wo.start)
        pl.when(j == 5)(d_wg.start)
        pl.when(j == 7)(d_wu.start)
        pl.when(j == 9)(d_wd.start)
        return carry

    d_k(0).wait()
    d_v(0).wait()
    prefetch(1)
    lax.fori_loop(0, HKV, att_body, 0)

    d_wmb.wait()
    d_wr.wait()
    d_wo.wait()
    d_wd.wait()
    mod_b = _rb(_dot(sc8, wmb_buf[...]))
    gb = mod_b[0:1, 3 * D:4 * D]
    gb_buf[...] = gb
    col_buf[0] = _col(mod_b[0:1, 0:D])
    col_buf[1] = _col(mod_b[0:1, D:2 * D])
    col_buf[2] = _col(_rb(1.0 + mod_b[0:1, 2 * D:3 * D]))
    col_buf[3] = _col(gb)
    col_buf[4] = _col(wr_buf[...].astype(F32).reshape(1, D))

    lane_id = lax.broadcasted_iota(jnp.int32, (1, TB), 1)

    NG = 8
    HG = HQ // NG
    CH = 8
    NC = D // CH
    NLB = OB // TB
    NOB = S // OB
    inv_d = np.float32(1.0 / D)
    eps_b = np.float32(np.float32(EPS).astype(jnp.bfloat16))

    def lanes(t):
        return slice(t * TB, (t + 1) * TB)

    def part_of(b, g):
        def tok2_of(h):
            return pl.ds(pl.multiple_of((h % 2) * (S // 2) + b * (OB // 2), OB // 2), OB // 2)
        heads = range(g * HG, (g + 1) * HG)
        o_cat = jnp.concatenate([as_bf16(o32[h // 2, tok2_of(h), :]) for h in heads], axis=1)
        wo_t = jnp.concatenate([as_bf16(wo32[h]) for h in heads], axis=1)
        return _dot(wo_t, o_cat, NT_DIMS)

    def accumulate(dst, src, part):
        for c in range(NC):
            r = slice(c * CH, (c + 1) * CH)
            dst[r, :] = part[r, :] if src is None else src[r, :] + part[r, :]

    def stage_a(p, att, x1_dst):
        means = []
        for t in range(NLB):
            acc = None
            for c in range(NC):
                r = slice(c * CH, (c + 1) * CH)
                c16 = slice((c // 2) * 16, (c // 2) * 16 + 16)
                xv = x_buf[p * NLB + t, c16, :].astype(F32)[(c % 2) * 8:(c % 2) * 8 + 8, :]
                x1 = _rb(xv + col_buf[0, r, :] * att[r, lanes(t)])
                x1_dst[r, lanes(t)] = x1
                acc = x1 if acc is None else acc + x1
            means.append(jnp.sum(acc, axis=0, keepdims=True) * inv_d)
        return means

    def stage_b(x1_src, means):
        invs = []
        for t in range(NLB):
            acc = None
            for c in range(NC):
                r = slice(c * CH, (c + 1) * CH)
                cen = x1_src[r, lanes(t)] - means[t]
                acc = cen * cen if acc is None else acc + cen * cen
            v = _rb(jnp.sum(acc, axis=0, keepdims=True) * inv_d)
            invs.append(1.0 / _rb(jnp.sqrt(_rb(v + eps_b))))
        return invs

    def stage_c(p, x1_src, means, invs, h_dst):
        mb = [_rb(m) for m in means]
        acc = [None] * NLB
        for c2 in range(NC // 2):
            for t in range(NLB):
                outs = []
                for c in (2 * c2, 2 * c2 + 1):
                    r = slice(c * CH, (c + 1) * CH)
                    x1 = x1_src[r, lanes(t)]
                    h2 = _rb(_rb(_rb(_rb(x1 - mb[t]) * invs[t]) * col_buf[2, r, :]) + col_buf[1, r, :])
                    tr = h2 * col_buf[4, r, :]
                    acc[t] = tr if acc[t] is None else acc[t] + tr
                    hb = h2 + h2 * 0.0
                    outs.append(x1 + _rb(col_buf[3, r, :] * hb))
                    h_dst[r, lanes(t)] = (lax.bitcast_convert_type(h2, jnp.int32)
                                          | lax.shift_right_logical(lax.bitcast_convert_type(x1, jnp.int32), 16))
                out_buf[p * NLB + t, 16 * c2:16 * c2 + 16, :] = jnp.concatenate(outs, axis=0).astype(BF16)
        return [_sort_key(_rb(jnp.sum(acc[t], axis=0, keepdims=True)), (p * NLB + t) * TB + lane_id)
                for t in range(NLB)]

    def stage_d(p, t, h_src):
        xh_buf[pl.ds(pl.multiple_of((p * NLB + t) * TB, TB), TB), :] = h_src[:, lanes(t)].T

    def merge_top(keys):
        cands = [top_buf[...]] + list(keys)
        top = jnp.zeros((1, TB), F32)
        for t in range(TOPK):
            m = jnp.max(functools.reduce(jnp.maximum, cands), axis=1, keepdims=True)
            top = jnp.where(lane_id == t, m, top)
            cands = [jnp.where(c_ == m, 0.0, c_) for c_ in cands]
        top_buf[...] = top

    WD_PER_BLOCK = -(-(F // 128) // (NOB - 1))

    def wd_transpose(i):
        cols = pl.ds(pl.multiple_of(i * 128, 128), 128)
        wdn_buf[cols, :] = wd_buf[:, cols].T

    def op_block(b, carry):
        p = b - 1
        z = b & 1
        bA, bB, bH = acc_buf.at[z], x1t_buf.at[z], h2t_buf.at[z]
        bX, bXn = att_buf.at[z], att_buf.at[1 - z]
        RA, RB = 2, 3
        cur = bA
        accumulate(bA, None, part_of(b, 0))
        means = stage_a(p, bX, bB)
        for g in range(1, NG - 1):
            if g == RA:
                accumulate(bX, cur, part_of(b, g))
                cur = bX
                invs = stage_b(bB, means)
            elif g == RB:
                keys = stage_c(p, bB, means, invs, bH)
                accumulate(bB, cur, part_of(b, g))
                cur = bB
            else:
                accumulate(cur, cur, part_of(b, g))
        for u in range(WD_PER_BLOCK):
            wd_transpose(jnp.minimum(p * WD_PER_BLOCK + u, F // 128 - 1))
        merge_top(keys)
        accumulate(bXn, cur, part_of(b, NG - 1))
        for t in range(NLB):
            stage_d(p, t, bH)
        for t in range(NLB):
            d_out(p * NLB + t).start()
        return carry

    top_buf[...] = jnp.zeros((1, TB), F32)
    accumulate(acc_buf.at[0], None, part_of(0, 0))
    for g in range(1, NG - 1):
        accumulate(acc_buf.at[0], acc_buf.at[0], part_of(0, g))
    accumulate(att_buf.at[1], acc_buf.at[0], part_of(0, NG - 1))
    lax.fori_loop(1, NOB, op_block, 0)
    zl = NOB & 1
    means = stage_a(NOB - 1, att_buf.at[zl], x1t_buf.at[zl])
    invs = stage_b(x1t_buf.at[zl], means)
    last_keys = stage_c(NOB - 1, x1t_buf.at[zl], means, invs, h2t_buf.at[zl])
    for t in range(NLB):
        d_out((NOB - 1) * NLB + t).start()

    top_bits = lax.bitcast_convert_type(top_buf[...], jnp.int32)
    for t in range(TOPK):
        top_smem[t] = top_bits[0, t]
    for t in range(NLB):
        key_buf[t:t + 1, :] = last_keys[t]

    def pull_cond(state):
        n, go = state
        return go

    def pull_body(state):
        n, _ = state
        kv = key_buf[...]
        m = jnp.max(jnp.max(kv, axis=0, keepdims=True), axis=1, keepdims=True)
        m_bits = lax.bitcast_convert_type(m, jnp.int32)[0, 0]
        slot = TOPK - 1 - n
        better = m_bits > top_smem[slot]

        @pl.when(better)
        def _():
            top_smem[slot] = m_bits
            key_buf[...] = jnp.where(kv == m, 0.0, kv)

        n1 = n + better.astype(jnp.int32)
        return n1, jnp.logical_and(better, n1 < TOPK)

    lax.while_loop(pull_cond, pull_body, (jnp.int32(0), jnp.bool_(True)))

    row8 = lax.broadcasted_iota(jnp.int32, (TOPK, 128), 0)
    kb = jnp.zeros((TOPK, 128), jnp.int32)
    idx = []
    for t in range(TOPK):
        kt = top_smem[t] - KEY_BIAS
        idx.append(jnp.clip((S - 1) - (kt & (S - 1)), 0, S - 1))
        kb = jnp.where(row8 == t, kt, kb)
    blk = [i // TB for i in idx]

    for t in range(NLB):
        hit = functools.reduce(jnp.logical_or, [b_ == (NOB - 1) * NLB + t for b_ in blk])
        pl.when(hit)(lambda t=t: stage_d(NOB - 1, t, h2t_buf.at[zl]))
    srt = lax.shift_right_logical(kb, 11)
    u16 = jnp.where(srt >= 0x8000, srt & 0x7FFF, 0xFFFF - srt)
    r_sel = lax.bitcast_convert_type(lax.shift_left(u16, 16), F32)[:, 0:1]

    for t in range(TOPK):
        xs_buf[pl.ds(t, 1), :] = xh_buf[pl.ds(idx[t], 1), :]
    xw = xs_buf[...]
    xs = lax.bitcast_convert_type(xw & jnp.int32(-65536), F32)
    x1s = lax.bitcast_convert_type(lax.shift_left(xw, 16), F32)
    xs_b = xs.astype(BF16)

    d_wg.wait()
    d_wu.wait()
    g = _rb(_dot(xs_b, wg_buf[...]))
    u = _rb(_dot(xs_b, wu_buf[...]))
    act = _rb(_rb(g * _sigmoid_b(g)) * u).astype(BF16)
    y = _rb(_dot(act, wdn_buf[...]))
    y = _rb(y * _sigmoid_b(r_sel))
    hb_sel = _rb(xs + _rb(_rb(xs * 0.0) + y))
    new = x1s + _rb(gb_buf[...] * hb_sel)
    new_t = jnp.concatenate([new, jnp.zeros((128 - TOPK, D), F32)], axis=0).T
    new_w = pltpu.bitcast(new_t.astype(BF16), jnp.int32)

    lane = lax.broadcasted_iota(jnp.int32, (D // 2, 128), 1)
    for b in range(NTB):
        d_out(b).wait()

    def d_patch(t):
        return cp(out_buf.at[blk[t]], out_hbm.at[:, pl.ds(pl.multiple_of(blk[t] * TB, TB), TB)], sem_patch.at[t])

    last = []
    for t in range(TOPK):
        f = blk[t] >= 0
        for t2 in range(t + 1, TOPK):
            f = jnp.logical_and(f, blk[t] != blk[t2])
        last.append(f)
    for t in range(TOPK):
        ln_t = idx[t] % TB
        rolled = pltpu.roll(new_w, (ln_t + (TB - t)) % TB, axis=1)
        out32[blk[t]] = jnp.where(lane == ln_t, rolled, out32[blk[t]])
        pl.when(last[t])(lambda t=t: d_patch(t).start())
    for t in range(TOPK):
        pl.when(last[t])(lambda t=t: d_patch(t).wait())


@jax.jit
def pallas_adaLN_cond__gqa_block_cached__moe_arch_mod__prompt_kernel(
    A_x, A_k_cache, A_v_cache, A_wq, A_wo, B_x, B_w_r, B_w_gate, B_w_up, B_w_down, c, w_mod,
):
    del B_x
    xt = A_x.reshape(S, D).T
    k = A_k_cache.reshape(HKV, S, DH)
    v = A_v_cache.reshape(HKV, S, DH)
    hbm = pl.BlockSpec(memory_space=pl.ANY)
    out = pl.pallas_call(
        _kernel,
        in_specs=[hbm] * 11,
        out_specs=hbm,
        out_shape=jax.ShapeDtypeStruct((D, S), BF16),
        scratch_shapes=[
            pltpu.VMEM((NTB, D, TB), BF16),
            pltpu.VMEM((NP, S, 128), BF16),
            pltpu.VMEM((S // 2, 128), BF16),
            pltpu.VMEM((2 * S, DH), BF16),
            pltpu.VMEM((HKV, S, DH), BF16),
            pltpu.VMEM((HKV, S, DH), BF16),
            pltpu.VMEM((HKV, D, 2 * DH), BF16),
            pltpu.VMEM((HQ, D, DH), BF16),
            pltpu.VMEM((D,), BF16),
            pltpu.VMEM((D, F), BF16),
            pltpu.VMEM((D, F), BF16),
            pltpu.VMEM((D, F), BF16),
            pltpu.VMEM((F, D), BF16),
            pltpu.VMEM((1, D), BF16),
            pltpu.VMEM((D, 2 * D), BF16),
            pltpu.VMEM((D, 4 * D), BF16),
            pltpu.VMEM((HKV, 2 * S, DH), BF16),
            pltpu.VMEM((S, D), jnp.int32),
            pltpu.VMEM((NTB, D, TB), BF16),
            pltpu.VMEM((OB // TB, TB), F32),
            pltpu.VMEM((1, TB), F32),
            pltpu.VMEM((2, D, OB), F32),
            pltpu.VMEM((2, D, OB), F32),
            pltpu.VMEM((2, D, OB), F32),
            pltpu.VMEM((2, D, OB), jnp.int32),
            pltpu.VMEM((5, D, TB), F32),
            pltpu.VMEM((1, D), F32),
            pltpu.VMEM((TOPK, D), jnp.int32),
            pltpu.SMEM((TOPK,), jnp.int32),
            pltpu.SemaphoreType.DMA((8,)),
            pltpu.SemaphoreType.DMA((HKV,)),
            pltpu.SemaphoreType.DMA((HKV,)),
            pltpu.SemaphoreType.DMA((HKV,)),
            pltpu.SemaphoreType.DMA((NTB,)),
            pltpu.SemaphoreType.DMA((NTB,)),
            pltpu.SemaphoreType.DMA((TOPK,)),
        ],
        compiler_params=pltpu.CompilerParams(vmem_limit_bytes=120 * 1024 * 1024, disable_bounds_checks=True,
                                             disable_semaphore_checks=True),
    )(xt, k, v, A_wq, A_wo.T, B_w_r, B_w_gate, B_w_up, B_w_down.T, c, w_mod)
    return out.T.reshape(1, S, D)
```
